```python
import os as _os
_os.environ.setdefault("JAX_PLATFORMS", "cpu")
import jax
import jax.numpy as jnp

def _softmax(x, axis=-1):
    return jax.nn.softmax(x, axis=axis)
def _gelu(x):
    return jax.nn.gelu(x, approximate=True)
def _silu(x):
    return jax.nn.silu(x)
def _sigmoid(x):
    return jax.nn.sigmoid(x)
def _layernorm(x, axis=-1, eps=1e-5):
    m = jnp.mean(x, axis=axis, keepdims=True)
    v = jnp.var(x, axis=axis, keepdims=True)
    return (x - m) / jnp.sqrt(v + eps)
def _scatter_add(tgt, idx, src, axis=0):
    return tgt.at[idx].add(src)
def _segment_sum(src, seg, n):
    return jax.ops.segment_sum(src, seg, n)
class _Rng:
    def __init__(self, key):
        self._k = key
    def _next(self):
        self._k, sub = jax.random.split(self._k)
        return sub
    def normal(self, shape):
        return jax.random.normal(self._next(), shape, dtype=jnp.bfloat16)
    def randint(self, lo, hi, shape):
        return jax.random.randint(self._next(), shape, lo, hi, dtype=jnp.int32)
    def uniform(self, shape, lo=0.0, hi=1.0):
        return jax.random.uniform(self._next(), shape, jnp.bfloat16, lo, hi)
    def permutation(self, n):
        return jax.random.permutation(self._next(), n)


kernel_name = 'sequential_preLN__sliding_block__glu_gated_glu__prompt'

def setup_inputs():
    _rng = _Rng(jax.random.key(int.from_bytes(__import__("os").urandom(4), "little")))
    _w = (lambda a: (lambda t: t.astype(jnp.bfloat16) if jnp.issubdtype(t.dtype, jnp.floating) else t)(jnp.asarray(a)))
    def _A_setup():
        B, S, D = 1, 2048, 640
        return {
            "x": _w((lambda *s: _rng.normal(s) * 0.05)(B, S, D)),
            "wqkv": _w((lambda *s: _rng.normal(s) * 0.05)(D, 3 * D)),
            "wo": _w((lambda *s: _rng.normal(s) * 0.05)(D, D)),
        }
    _A_in = _A_setup()

    def _B_setup():
        B, S, D, F = 1, 2048, 640, 1728
        return {
            "x": _w((lambda *s: _rng.normal(s) * 0.05)(B, S, D)),
            "w_gate": _w((lambda *s: _rng.normal(s) * 0.05)(D, F)),
            "w_up": _w((lambda *s: _rng.normal(s) * 0.05)(D, F)),
            "w_down": _w((lambda *s: _rng.normal(s) * 0.05)(F, D)),
        }
    _B_in = _B_setup()

    return {
        "A_x": _A_in["x"],
        "A_wqkv": _A_in["wqkv"],
        "A_wo": _A_in["wo"],
        "B_x": _B_in["x"],
        "B_w_gate": _B_in["w_gate"],
        "B_w_up": _B_in["w_up"],
        "B_w_down": _B_in["w_down"],
    }

def reference(A_x, A_wqkv, A_wo, B_x, B_w_gate, B_w_up, B_w_down):
    def _A_ref(x, wqkv, wo):
        B, S, D = x.shape
        H = 32; Dh = D // H; W = 256
        qkv = (lambda x, *d: x.transpose(*d))((x @ wqkv).reshape(B, S, 3, H, Dh), 2, 0, 3, 1, 4)
        q, k, v = qkv[0], qkv[1], qkv[2]
        scores = jnp.einsum("bhqd,bhkd->bhqk", q, k) * (Dh ** -0.5)
        idx = jnp.arange(S)
        mask = (idx[:, None] - idx[None, :] >= 0) & (idx[:, None] - idx[None, :] < W)
        scores = jnp.where(mask[None, None], scores, -1e9)
        p = _softmax(scores, axis=-1)
        o = jnp.einsum("bhqk,bhkd->bhqd", p, v)
        return (lambda x, *d: x.transpose(*d))(o, 0, 2, 1, 3).reshape(B, S, D) @ wo

    def _B_ref(x, w_gate, w_up, w_down):
        g = jnp.einsum("bsd,df->bsf", x, w_gate)
        u = jnp.einsum("bsd,df->bsf", x, w_up)
        h = _sigmoid(g) * u
        return jnp.einsum("bsf,fd->bsd", h, w_down)

    x = A_x
    h = x + _A_ref(_layernorm(x, axis=-1), A_wqkv, A_wo)
    h2 = h + _B_ref(_layernorm(h, axis=-1), B_w_gate, B_w_up, B_w_down)
    return h2
```

```python
import functools
import math
import os

import jax
import jax.numpy as jnp
from jax import lax
import jax.experimental.pallas as pl
import jax.experimental.pallas.tpu as pltpu

S, D, H, DH, W, F = 2048, 640, 32, 20, 256, 1728
T = 256
NB = S // T
NQT = T // 128
NG = H // 4
NP = H // 2
FT = F // 128
FM = FT * 128
NEG = -1e9
EPS = 1e-5
f32, bf16, u32 = jnp.float32, jnp.bfloat16, jnp.uint32
NT = (((1,), (1,)), ((), ()))
_E = lambda k, d: int(os.environ.get(k, d))
CSTAR = _E("CSTAR", 3)
TAIL0 = _E("TAIL0", 1)
TAIL1 = _E("TAIL1", 2)
TAIL2 = _E("TAIL2", 2)
NSB = _E("NSB", 2)
PSTAGE = _E("PSTAGE", 0)
SPREAD = _E("SPREAD", 1)
PBF = _E("PBF", 1)


def _ln(x):
    m = jnp.mean(x, axis=-1, keepdims=True)
    xc = x - m
    v = jnp.mean(xc * xc, axis=-1, keepdims=True)
    return xc * lax.rsqrt(v + EPS)


def _sel(mask, a, b):
    if a is None and b is None:
        return None
    if a is None:
        a = jnp.zeros_like(b)
    if b is None:
        b = jnp.zeros_like(a)
    return jnp.where(mask, a, b)


def _sigmoid(x):
    return 0.5 * jnp.tanh(0.5 * x) + 0.5


def _dot(a, b):
    return jnp.dot(a, b, preferred_element_type=f32)


def _dot_nt(a, b):
    return lax.dot_general(a, b, NT, preferred_element_type=f32)


def _proj_chunks(lhs, tiles, done, put, get):
    chunks = []

    def tail(group):
        def run():
            a = lhs()[:, 512:D]
            for slot, (key, fn) in enumerate(group):
                if len(group) == 4:
                    put(slot, fn(a, 512, D))
                else:
                    q = T // 4
                    put(slot, jnp.concatenate(
                        [fn(a[r * q:(r + 1) * q], 512, D) for r in range(4)], axis=0))
        return run

    def head(slot, key, fn):
        def run():
            done(key, get(slot) + fn(lhs()[:, 0:512], 0, 512))
        return run

    for i in range(0, len(tiles), 4):
        group = tiles[i:i + 4]
        chunks.append(tail(group))
        chunks += [head(slot, key, fn) for slot, (key, fn) in enumerate(group)]
    return chunks


def _once(fn):
    cache = []

    def get():
        if not cache:
            cache.append(fn())
        return cache[0]
    return get


def _kernel(x_hbm, wqkv_hbm, wo_hbm, wg_hbm, wu_hbm, wd_hbm, o_ref,
            xs, wqkv, wo, wgu, wd, sems, xsems,
            xn_scr, q_scr, k_scr, vt_scr, ot_scr, o_scr, h_scr, hn_scr, act_scr, *bufs):
    step = pl.program_id(0)
    s_scr, p_scr, a_scr, t_scr = bufs[:NSB], bufs[NSB:NSB + 3], bufs[NSB + 3:NSB + 5], bufs[NSB + 5:]
    zw = lax.shift_right_logical(step, 8)
    zr = lax.shift_right_logical(step, 9)

    def put(slot, val):
        t_scr[slot][zw] = val

    def get(slot):
        return t_scr[slot][zr]

    copies = dict(
        wv=pltpu.make_async_copy(wqkv_hbm.at[:, 2 * D:3 * D], wqkv.at[:, 2 * D:3 * D], sems.at[0]),
        wk=pltpu.make_async_copy(wqkv_hbm.at[:, D:2 * D], wqkv.at[:, D:2 * D], sems.at[1]),
        wq=pltpu.make_async_copy(wqkv_hbm.at[:, 0:D], wqkv.at[:, 0:D], sems.at[2]),
        wo=pltpu.make_async_copy(wo_hbm, wo, sems.at[3]),
        wg=pltpu.make_async_copy(wg_hbm.at[0:FM], wgu.at[0:FM], sems.at[4]),
        wu=pltpu.make_async_copy(wu_hbm.at[0:FM], wgu.at[FM:2 * FM], sems.at[5]),
        wg2=pltpu.make_async_copy(wg_hbm.at[FM:F], wgu.at[2 * FM:2 * FM + 64], sems.at[6]),
        wu2=pltpu.make_async_copy(wu_hbm.at[FM:F], wgu.at[2 * FM + 64:2 * F], sems.at[7]),
        wd=pltpu.make_async_copy(wd_hbm, wd, sems.at[8]),
    )

    def rows_of(b):
        return pl.ds(b * T if isinstance(b, int) else pl.multiple_of(b * T, T), T)

    def xcopy(b):
        return pltpu.make_async_copy(x_hbm.at[rows_of(b)], xs.at[rows_of(b)], xsems.at[b])

    def body(first, last):
        blk = 0 if first else step

        sub8 = lax.broadcasted_iota(jnp.int32, (8, 128), 0)
        lo4 = sub8 < 4
        lane16 = lax.broadcasted_iota(jnp.int32, (16, 128), 1)
        lane32 = lax.broadcasted_iota(jnp.int32, (32, 128), 1)
        m_s1 = (lane32 & 32) != 0
        m_s2 = (lane32 & 64) != 0
        r32 = lax.broadcasted_iota(jnp.int32, (32, 128), 0)
        tri_first = r32 > (lane32 & 31)
        laneT = lax.broadcasted_iota(jnp.int32, (T, 128), 1)

        def qkv_chunks(xn, which):
            got = {}
            qscale = (DH ** -0.5) * math.log2(math.e)

            def done(key, val):
                name, n = key
                if name == "v":
                    for c in range(NQT):
                        vt = val[c * 128:(c + 1) * 128, :].T
                        for i in range(16):
                            r = 16 * n + i
                            p, e = divmod(r, 5)
                            piece = vt[8 * i:8 * i + 8]
                            kt = blk * NQT + c
                            if e == 2:
                                vt_scr[kt, 48 * p + 16:48 * p + 24, :] = jnp.where(lo4, piece, 1.0)
                                vt_scr[kt, 48 * p + 24:48 * p + 32, :] = jnp.where(lo4, 1.0, piece)
                            else:
                                o = 48 * p + 8 * (e if e < 2 else e + 1)
                                vt_scr[kt, o:o + 8, :] = piece
                    return
                if name == "q":
                    val = val * qscale
                got[key] = val
                for g in range(NG):
                    lo = 80 * g
                    t0, t1 = lo // 128, (lo + 79) // 128
                    if t1 != n:
                        continue
                    tile = val if t0 == t1 else jnp.where(laneT >= lo % 128, got[(name, t0)], val)
                    if name == "q":
                        q_scr[g] = tile.astype(bf16)
                    else:
                        k_scr[g, rows_of(blk), :] = tile.astype(bf16)

            base = {"q": 0, "k": D, "v": 2 * D}
            tiles = []
            for name in which:
                for n in range(5):
                    c0 = base[name] + 128 * n
                    tiles.append(((name, n),
                                  lambda a, k0, k1, c0=c0: _dot(a, wqkv[k0:k1, c0:c0 + 128])))
            return _proj_chunks(xn, tiles, done, put, get)

        def gu_chunks(hn, g0, g1):
            gate = {}

            def done(key, val):
                name, f = key
                if name == "g":
                    put(4, _sigmoid(val))
                elif name == "u":
                    act_scr[:, f * 128:(f + 1) * 128] = (get(4) * val).astype(bf16)
                else:
                    a = _sigmoid(val) * pltpu.roll(val, 64, 1)
                    act_scr[:, FM:F] = a[:, 0:64].astype(bf16)

            tiles = []
            for f in range(FT):
                for name, r0 in (("g", f * 128), ("u", FM + f * 128)):
                    tiles.append(((name, f),
                                  lambda a, k0, k1, r0=r0: _dot_nt(a, wgu[r0:r0 + 128, k0:k1])))
            tiles.append((("gu", FT), lambda a, k0, k1: _dot_nt(a, wgu[2 * FM:2 * F, k0:k1])))
            return _proj_chunks(hn, tiles[4 * g0:4 * g1], done, put, get)

        def down_chunks():
            ppar = (step + 1) % 2

            def d_chunk(n0, n1, k0, k1, nsplit=1):
                def run():
                    cols = slice(n0 * 128, n1 * 128)
                    q = T // nsplit
                    for r in range(nsplit):
                        rows = slice(r * q, (r + 1) * q)
                        y = h_scr[ppar, rows, cols] + _dot(act_scr[rows, k0:k1], wd[k0:k1, cols])
                        if k1 == F:
                            o_ref[rows, cols] = y.astype(o_ref.dtype)
                        else:
                            h_scr[ppar, rows, cols] = y
                return run

            chunks = []
            for k in (0, 512, 1024):
                chunks += [d_chunk(n, n + 1, k, k + 512) for n in range(5)]
            chunks += [d_chunk(0, 2, 1536, F), d_chunk(2, 4, 1536, F), d_chunk(4, 5, 1536, F, 2)]
            return chunks

        dq = []
        if not first:
            dq += gu_chunks(_once(lambda: hn_scr[...]), CSTAR, 7) + down_chunks()

        def run(n, keep=0):
            for _ in range(n):
                if len(dq) > keep:
                    dq.pop(0)()

        if last:
            run(len(dq))
            return

        if first:
            xcopy(0).start()
            for name in ("wv", "wk", "wq", "wo"):
                copies[name].start()
            xcopy(1).start()
            for name in ("wg", "wu", "wg2", "wu2", "wd"):
                copies[name].start()
            for b in range(2, NB):
                xcopy(b).start()
            xcopy(0).wait()
            xnv = _ln(xs[rows_of(0), :].astype(f32)).astype(bf16)
            for name in "vkq":
                copies["w" + name].wait()
                for ch in qkv_chunks(lambda: xnv, name):
                    ch()
        else:
            @pl.when(step < NB - 1)
            def _():
                xcopy(step + 1).wait()
            for ch in qkv_chunks(_once(lambda: xn_scr[...]), "vkq"):
                ch()
        run(TAIL0)

        row0 = 0 if first else pl.multiple_of(step * T, T)
        kt0 = blk * NQT
        tmin = lambda c: max(0, 8 - 4 * c) if first else 0

        def qk(c, g, buf):
            ms = []
            for j in range(4):
                t0, t1 = max(j, tmin(c)), j + 9
                rows = (t1 - t0) * 32
                start = row0 + (c * 128 - 256 + t0 * 32)
                if not first:
                    start = pl.multiple_of(start, 32)
                kwin = k_scr[g, pl.ds(start, rows), :]
                qb = pltpu.bitcast(q_scr[g, c * 128 + j * 32:c * 128 + (j + 1) * 32, :], u32)
                slots = []
                for s in range(4):
                    h = s ^ j
                    lo = (80 * g + 20 * h) % 128
                    inh = ((lane16 - lo) & 127) < 20
                    slots.append(jnp.where(inh, qb, jnp.zeros_like(qb)))
                qm = pltpu.bitcast(jnp.concatenate(slots, axis=0), bf16)
                st = _dot_nt(kwin, qm)
                parts = []
                if t0 == j:
                    parts.append(jnp.where(tri_first, st[0:32], NEG))
                    if rows > 64:
                        parts.append(st[32:rows - 32])
                elif rows > 32:
                    parts.append(st[0:rows - 32])
                parts.append(jnp.where(tri_first, NEG, st[rows - 32:rows]))
                st = jnp.concatenate(parts, axis=0)
                ms.append(jnp.max(st, axis=0, keepdims=True))
                s_scr[buf][zw, j, t0 * 32:t1 * 32, :] = st
            return ms

        def probs(kt, sbuf, ms):
            ph = [[] for _ in range(4)]
            for t in range(4 * kt, 4 * kt + 4):
                p = []
                for j in range(4):
                    if j <= t <= j + 8:
                        p.append(jnp.exp2(s_scr[sbuf][zr, j, t * 32:(t + 1) * 32, :] - ms[j]))
                    else:
                        p.append(None)
                u = [_sel(m_s1, p[j ^ 1], p[j]) for j in range(4)]
                for h in range(4):
                    ph[h].append(_sel(m_s2, u[h ^ 2], u[h]))
            return [jnp.concatenate(ph[h], axis=0) for h in range(4)]

        def softmax(c, sbuf, ms):
            for kt in range(tmin(c) // 4, 3):
                for h, p in enumerate(probs(kt, sbuf, ms)):
                    p_scr[kt][zw, h] = p

        def pv(c, g, kt, sbuf, ms):
            if PSTAGE:
                ps = [p_scr[kt][zr, h] for h in range(4)]
            else:
                ps = probs(kt, sbuf, ms)
            res = []
            for h in range(4):
                r0 = 48 * (2 * g + h // 2) + 24 * (h % 2)
                r = _dot(vt_scr[kt0 + c - 2 + kt, r0:r0 + 24, :], ps[h].astype(bf16) if PBF else ps[h])
                if kt > tmin(c) // 4:
                    r = r + a_scr[kt - 1][zr, h]
                if kt < 2:
                    a_scr[kt][zw, h] = r
                res.append(r)
            if kt < 2:
                return
            for pp in range(2):
                re, ro = res[2 * pp], res[2 * pp + 1]
                a, b = re[16:24], ro[0:8]
                inv = pl.reciprocal(jnp.where(lo4, b, a), approx=True)
                inv_r = pltpu.roll(inv, 4, 0)
                ie = jnp.where(lo4, inv_r, inv)
                io = jnp.where(lo4, inv, inv_r)
                mid = jnp.where(lo4, a, b) * inv_r
                blkv = jnp.concatenate(
                    [re[0:8] * ie, re[8:16] * ie, mid, ro[8:16] * io, ro[16:24] * io], axis=0)
                pair = 2 * g + pp
                ot_scr[c, 40 * pair:40 * pair + 40, :] = blkv
            if g == NG - 1:
                finish(c)

        def finish(c):
            o = ot_scr[c].T
            lane = lax.broadcasted_iota(jnp.int32, (32, D), 1)
            hl = (lane * 3277) >> 16
            h1 = (hl & 1) != 0
            h2 = (hl & 2) != 0
            b4 = [o[32 * j:32 * (j + 1)] for j in range(4)]
            u = [jnp.where(h1, b4[j ^ 1], b4[j]) for j in range(4)]
            out = [jnp.where(h2, u[j ^ 2], u[j]) for j in range(4)]
            o_scr[c * 128:(c + 1) * 128, :] = jnp.concatenate(out, axis=0).astype(bf16)

        items = [(c, g) for c in range(NQT) for g in range(NG)]
        n = len(items)
        keep = TAIL1 + TAIL2
        navail = max(len(dq) - keep, 0)
        nslots = n + 1
        ms = {}
        for i in range(nslots):
            if PSTAGE and 0 <= i - 1 < n:
                softmax(items[i - 1][0], (i - 1) % NSB, ms[i - 1])
            if i < n:
                ms[i] = qk(*items[i], i % NSB)
            nd = ((i + 1) * navail) // nslots - (i * navail) // nslots
            if i == 0:
                run(nd, keep)
                continue
            c, g = items[i - 1]
            kts = list(range(tmin(c) // 4, 3))
            if SPREAD:
                pre = [0] * len(kts)
                order = list(range(1, len(kts))) + [0] if i < n else list(range(len(kts)))
                for q in range(nd):
                    pre[order[q % len(kts)]] += 1
            else:
                pre = [nd] + [0] * (len(kts) - 1)
            for kt, m in zip(kts, pre):
                run(m, keep)
                pv(c, g, kt, (i - 1) % NSB, ms[i - 1])
        run(TAIL1)

        if first:
            copies["wo"].wait()
        hs = {}

        def h_done(n, val):
            hs[n] = xs[rows_of(blk), n * 128:(n + 1) * 128].astype(f32) + val
            h_scr[blk % 2, :, n * 128:(n + 1) * 128] = hs[n]

        tiles = [(n, lambda a, k0, k1, n=n: _dot(a, wo[k0:k1, n * 128:(n + 1) * 128]))
                 for n in range(5)]
        for ch in _proj_chunks(_once(lambda: o_scr[...]), tiles, h_done, put, get):
            ch()
        h = jnp.concatenate([hs[n] for n in range(5)], axis=1)
        hnv = _ln(h).astype(bf16)
        hn_scr[...] = hnv
        run(len(dq))
        if first:
            xcopy(1).wait()
            for name in ("wg", "wu", "wg2", "wu2"):
                copies[name].wait()
        nb = 1 if first else jnp.minimum(step + 1, NB - 1)
        gch = gu_chunks(lambda: hnv, 0, CSTAR)
        for ch in gch[:2]:
            ch()
        xn_scr[...] = _ln(xs[rows_of(nb), :].astype(f32)).astype(bf16)
        for ch in gch[2:]:
            ch()
        if first:
            copies["wd"].wait()

    @pl.when(step == 0)
    def _():
        with jax.named_scope("S_first"):
            body(True, False)

    @pl.when(jnp.logical_and(step > 0, step < NB))
    def _():
        with jax.named_scope("S_mid"):
            body(False, False)

    @pl.when(step == NB)
    def _():
        with jax.named_scope("S_last"):
            body(False, True)


@jax.jit
def pallas_sequential_preLN__sliding_block__glu_gated_glu__prompt_kernel(
    A_x, A_wqkv, A_wo, B_x, B_w_gate, B_w_up, B_w_down):
    del B_x
    x = A_x.reshape(S, D)
    hbm = pl.BlockSpec(memory_space=pl.ANY)
    out = pl.pallas_call(
        _kernel,
        grid=(NB + 1,),
        in_specs=[hbm] * 6,
        out_specs=pl.BlockSpec((T, D), lambda i: (jnp.maximum(i - 1, 0), 0)),
        out_shape=jax.ShapeDtypeStruct((S, D), bf16),
        scratch_shapes=[
            pltpu.VMEM((S, D), bf16),
            pltpu.VMEM((D, 3 * D), bf16),
            pltpu.VMEM((D, D), bf16),
            pltpu.VMEM((2 * F, D), bf16),
            pltpu.VMEM((F, D), bf16),
            pltpu.SemaphoreType.DMA((9,)),
            pltpu.SemaphoreType.DMA((NB,)),
            pltpu.VMEM((T, D), bf16),
            pltpu.VMEM((NG, T, 128), bf16),
            pltpu.VMEM((NG, S, 128), bf16),
            pltpu.VMEM((S // 128, 48 * NP, 128), f32),
            pltpu.VMEM((NQT, D, 128), f32),
            pltpu.VMEM((T, D), bf16),
            pltpu.VMEM((2, T, D), f32),
            pltpu.VMEM((T, D), bf16),
            pltpu.VMEM((T, F), bf16),
        ] + [pltpu.VMEM((1, 4, 384, 128), f32)] * NSB + [pltpu.VMEM((1, 4, 128, 128), f32)] * 3
        + [pltpu.VMEM((1, 4, 24, 128), f32)] * 2 + [pltpu.VMEM((1, T, 128), f32)] * 5,
        compiler_params=pltpu.CompilerParams(
            dimension_semantics=("arbitrary",),
            vmem_limit_bytes=100 * 1024 * 1024),
        name="fused_block",
    )(x, A_wqkv, A_wo, B_w_gate.T, B_w_up.T, B_w_down)
    return out.reshape(1, S, D)
```

```python
import functools
import math

import jax
import jax.numpy as jnp
from jax import lax
import jax.experimental.pallas as pl
import jax.experimental.pallas.tpu as pltpu

S, D, H, DH, F = 2048, 640, 32, 20, 1728
T = 256
NB = S // T
NQT = T // 128
NG = H // 4
NP = H // 2
FT = F // 128
FM = FT * 128
NEG = -1e9
EPS = 1e-5
QSCALE = (DH ** -0.5) * math.log2(math.e)
f32, bf16, u32 = jnp.float32, jnp.bfloat16, jnp.uint32

FA = 256
HEAD, TAIL1, TAIL2 = 3, 2, 2
HEAD0, TAIL10, TAIL20 = 1, 2, 2
KA = 2
WAIT_AT = 5
UNITS = ("k0", "q0", "k1", "q1", "k2", "v0", "v1", "v2", "q2")
LN_AT = (0, 10, 30)


def _ln(x):
    m = jnp.mean(x, axis=-1, keepdims=True)
    xc = x - m
    v = jnp.mean(xc * xc, axis=-1, keepdims=True)
    return xc * lax.rsqrt(v + EPS)


def _sel(mask, a, b):
    if a is None and b is None:
        return None
    if a is None:
        a = jnp.zeros_like(b)
    if b is None:
        b = jnp.zeros_like(a)
    return jnp.where(mask, a, b)


def _sigmoid(x):
    return 0.5 * jnp.tanh(0.5 * x) + 0.5


def _dot(a, b):
    return jnp.dot(a, b, preferred_element_type=f32)


def _dot_nt(a, b):
    return lax.dot_general(a, b, (((1,), (1,)), ((), ())), preferred_element_type=f32)


def _proj_chunks(tiles, put, get):
    chunks = []

    def tail(group):
        def run():
            ns = {4: 1, 2: 2}.get(len(group), 4)
            q = T // ns
            for slot, (lhs, fn, _) in enumerate(group):
                a = lhs(512, D)
                put(slot, jnp.concatenate(
                    [fn(a[r * q:(r + 1) * q], 512, D) for r in range(ns)], axis=0))
        return run

    def head(slot, lhs, fn, done):
        def run():
            done(get(slot) + fn(lhs(0, 512), 0, 512))
        return run

    for i in range(0, len(tiles), 4):
        group = tiles[i:i + 4]
        chunks.append(tail(group))
        chunks += [head(slot, *tile) for slot, tile in enumerate(group)]
    return chunks


def _lazy_cols(fn):
    cache = []

    def get(k0, k1):
        if not cache:
            cache.append(fn())
        return cache[0][:, k0:k1]
    return get


def _kernel(x_hbm, wqkv_hbm, wo_hbm, wg_hbm, wu_hbm, wd_hbm, o_hbm,
            ob, xs, wqkv, wo, wgu, wd, sems,
            q_scr, k_scr, vt_scr, ot_scr, o_scr, h_scr, hn_scr, act_scr, *bufs):
    step = pl.program_id(0)
    s_scr, g_scr = bufs[0:2], bufs[2]
    sets, xn_scr = [bufs[3:7], bufs[7:11]], bufs[11:14]
    a_scr = xn_scr
    zw = lax.shift_right_logical(step, 8)
    zr = lax.shift_right_logical(step, 9)

    def stage(k):
        def put(slot, val):
            sets[k][slot][zw] = val

        def get(slot):
            return sets[k][slot][zr]
        return put, get

    cp = pltpu.make_async_copy
    ka = D + 128 * KA
    copies = dict(
        x0=cp(x_hbm.at[0:T], xs.at[0, 0:T], sems.at[0]),
        x1=cp(x_hbm.at[T:2 * T], xs.at[0, T:2 * T], sems.at[1]),
        wka=cp(wqkv_hbm.at[:, D:ka], wqkv.at[:, D:ka], sems.at[2]),
        wkb=cp(wqkv_hbm.at[:, ka:2 * D], wqkv.at[:, ka:2 * D], sems.at[3]),
        wq=cp(wqkv_hbm.at[:, 0:D], wqkv.at[:, 0:D], sems.at[4]),
        wv=cp(wqkv_hbm.at[:, 2 * D:3 * D], wqkv.at[:, 2 * D:3 * D], sems.at[5]),
        wo=cp(wo_hbm, wo, sems.at[6]),
        wga=cp(wg_hbm.at[0:FA], wgu.at[0:FA], sems.at[6]),
        wua=cp(wu_hbm.at[0:FA], wgu.at[FM:FM + FA], sems.at[6]),
        x2=cp(x_hbm.at[2 * T:3 * T], xs.at[0, 2 * T:3 * T], sems.at[6]),
        x35=cp(x_hbm.at[3 * T:6 * T], xs.at[0, 3 * T:6 * T], sems.at[7]),
        wg2=cp(wg_hbm.at[FM:F], wgu.at[2 * FM:2 * FM + 64], sems.at[8]),
        wu2=cp(wu_hbm.at[FM:F], wgu.at[2 * FM + 64:2 * F], sems.at[8]),
        wgb=cp(wg_hbm.at[FA:FM], wgu.at[FA:FM], sems.at[8]),
        wub=cp(wu_hbm.at[FA:FM], wgu.at[FM + FA:2 * FM], sems.at[8]),
        wd=cp(wd_hbm, wd, sems.at[8]),
        x67=cp(x_hbm.at[6 * T:8 * T], xs.at[0, 6 * T:8 * T], sems.at[8]),
    )

    def rows_of(b, n=T):
        return pl.ds(b * T if isinstance(b, int) else pl.multiple_of(b * T, T), n)

    def ocopy(b):
        return cp(ob.at[rows_of(b)], o_hbm.at[rows_of(b)], sems.at[0])

    def ocopy_last(n):
        rows, cols = rows_of(NB - 1), pl.ds(n * 128, 128)
        return cp(ob.at[rows, cols], o_hbm.at[rows, cols], sems.at[0])

    lo4 = lax.broadcasted_iota(jnp.int32, (8, 128), 0) < 4

    def qkv_tiles(b, xn, which, hook=None):
        got = {}
        lane = lax.broadcasted_iota(jnp.int32, (T, 128), 1)

        def done(key, val):
            name, n = key
            if hook:
                hook(val)
            if name == "v":
                for c in range(NQT):
                    vt = val[c * 128:(c + 1) * 128, :].T
                    for i in range(16):
                        p, e = divmod(16 * n + i, 5)
                        piece = vt[8 * i:8 * i + 8]
                        kt = b * NQT + c
                        if e == 2:
                            vt_scr[kt, 48 * p + 16:48 * p + 24, :] = jnp.where(lo4, piece, 1.0)
                            vt_scr[kt, 48 * p + 24:48 * p + 32, :] = jnp.where(lo4, 1.0, piece)
                        else:
                            o = 48 * p + 8 * (e if e < 2 else e + 1)
                            vt_scr[kt, o:o + 8, :] = piece
                return
            if name == "q":
                val = val * QSCALE
            got[key] = val
            for g in range(NG):
                lo = 80 * g
                t0, t1 = lo // 128, (lo + 79) // 128
                if t1 != n:
                    continue
                tile = val if t0 == t1 else jnp.where(lane >= lo % 128, got[(name, t0)], val)
                if name == "q":
                    q_scr[g, rows_of(b), :] = tile.astype(bf16)
                else:
                    k_scr[g, rows_of(b), :] = tile

        base = {"q": 0, "k": D, "v": 2 * D}
        tiles = []
        for name in which:
            for n in range(5):
                c0 = base[name] + 128 * n
                tiles.append((xn, lambda a, k0, k1, c0=c0: _dot(a, wqkv[k0:k1, c0:c0 + 128]),
                              functools.partial(done, (name, n))))
        return tiles

    def ln1_part(b, r, part):
        rows = slice(part * T // 4, (part + 1) * T // 4)
        xn_scr[r][zw, rows, :] = _ln(xs.at[zr, rows_of(b)][rows, :].astype(f32))

    def gu_chunks(hn, head):
        def done(key, val):
            name, f = key
            if name == "g":
                g_scr[zw] = _sigmoid(val)
            elif name == "u":
                act_scr[:, f * 128:(f + 1) * 128] = g_scr[zr] * val
            else:
                act_scr[:, FM:F] = (_sigmoid(val) * pltpu.roll(val, 64, 1))[:, 0:64]

        tiles = []
        for f in range(FT):
            for name, r0 in (("g", f * 128), ("u", FM + f * 128)):
                tiles.append((hn, lambda a, k0, k1, r0=r0: _dot_nt(a, wgu[r0:r0 + 128, k0:k1]),
                              functools.partial(done, (name, f))))
        tiles.append((hn, lambda a, k0, k1: _dot_nt(a, wgu[2 * FM:2 * F, k0:k1]),
                      functools.partial(done, ("gu", FT))))
        return _proj_chunks(tiles[:FA // 64] if head else tiles[FA // 64:], *stage(0))

    def deferred(last=False):
        par = (step + 1) % 2

        def d_chunk(n0, n1, k0, k1, nsplit=1, then=None):
            def run():
                cols = slice(n0 * 128, n1 * 128)
                q = T // nsplit
                for r in range(nsplit):
                    rows = slice(r * q, (r + 1) * q)
                    y = h_scr[par, rows, cols] + _dot(act_scr[rows, k0:k1], wd[k0:k1, cols])
                    if k1 == F:
                        ob.at[rows_of(step - 1)][rows, cols] = y.astype(bf16)
                    else:
                        h_scr[par, rows, cols] = y
                if then:
                    then().start()
            return run

        early = [d_chunk(0, 2, 0, 256), d_chunk(2, 4, 0, 256), d_chunk(4, 5, 0, 256, 2)]
        ks = ((256, 768), (768, 1280), (1280, F))
        if last:
            late = [d_chunk(n, n + 1, k0, k1,
                            then=functools.partial(ocopy_last, n) if k1 == F else None)
                    for n in range(5) for k0, k1 in ks]
        else:
            late = [d_chunk(n, n + 1, k0, k1,
                            then=(lambda: ocopy(step - 1)) if (k1 == F and n == 4) else None)
                    for k0, k1 in ks for n in range(5)]
        return early + gu_chunks(_lazy_cols(lambda: hn_scr[...]), False) + late

    def main(first, dq):
        blk = 0 if first else step
        lane16 = lax.broadcasted_iota(jnp.int32, (16, 128), 1)
        lane32 = lax.broadcasted_iota(jnp.int32, (32, 128), 1)
        m_s1 = (lane32 & 32) != 0
        m_s2 = (lane32 & 64) != 0
        tri_first = lax.broadcasted_iota(jnp.int32, (32, 128), 0) > (lane32 & 31)
        kv = k_scr if first else k_scr.at[:, rows_of(step - 1, 2 * T)]
        koff = -T if first else 0
        qv = q_scr.at[:, rows_of(blk)]
        kt0 = blk * NQT
        tmin = lambda c: max(0, 8 - 4 * c) if first else 0
        soff = lambda c: -8 if first and c == 0 else 0

        def run(n, keep=0):
            for _ in range(n):
                if len(dq) > keep:
                    dq.pop(0)()

        def qk(c, g, buf):
            ms = {}
            for j in (3, 2, 1, 0):
                t0, t1 = max(j, tmin(c)), j + 9
                rows = (t1 - t0) * 32
                start = koff + c * 128 + t0 * 32
                qb = pltpu.bitcast(qv[g, c * 128 + j * 32:c * 128 + (j + 1) * 32, :], u32)
                slots = []
                for s in range(4):
                    lo = (80 * g + 20 * (s ^ j)) % 128
                    slots.append(jnp.where(((lane16 - lo) & 127) < DH, qb, jnp.zeros_like(qb)))
                qm = pltpu.bitcast(jnp.concatenate(slots, axis=0), bf16)
                st = _dot_nt(kv[g, start:start + rows, :], qm)
                parts = []
                if t0 == j:
                    parts.append(jnp.where(tri_first, st[0:32], NEG))
                    parts.append(st[32:rows - 32])
                elif rows > 32:
                    parts.append(st[0:rows - 32])
                parts.append(jnp.where(tri_first, NEG, st[rows - 32:rows]))
                st = jnp.concatenate(parts, axis=0)
                ms[j] = jnp.max(st, axis=0, keepdims=True)
                s_scr[buf][zw, j, (t0 + soff(c)) * 32:(t1 + soff(c)) * 32, :] = st
            return ms

        def probs(c, kt, sbuf, ms):
            ph = [[] for _ in range(4)]
            for t in range(4 * kt, 4 * kt + 4):
                ts = t + soff(c)
                p = [jnp.exp2(s_scr[sbuf][zr, j, ts * 32:(ts + 1) * 32, :] - ms[j])
                     if j <= t <= j + 8 else None for j in range(4)]
                u = [_sel(m_s1, p[j ^ 1], p[j]) for j in range(4)]
                for h in range(4):
                    ph[h].append(_sel(m_s2, u[h ^ 2], u[h]))
            return [jnp.concatenate(ph[h], axis=0).astype(bf16) for h in range(4)]

        def pv(c, g, kt, sbuf, ms):
            ps = probs(c, kt, sbuf, ms)
            res = []
            for h in range(4):
                r0 = 48 * (2 * g + h // 2) + 24 * (h % 2)
                r = _dot(vt_scr[kt0 + c - 2 + kt, r0:r0 + 24, :], ps[h])
                if kt > tmin(c) // 4:
                    r = r + a_scr[kt - 1][zr, T:T + 24, h * 128:(h + 1) * 128]
                if kt < 2:
                    a_scr[kt][zw, T:T + 24, h * 128:(h + 1) * 128] = r
                res.append(r)
            if kt < 2:
                return
            for pp in range(2):
                re, ro = res[2 * pp], res[2 * pp + 1]
                a, b = re[16:24], ro[0:8]
                l = jnp.where(lo4, b, a)
                inv = pl.reciprocal(l, approx=True)
                inv = inv * (2.0 - l * inv)
                inv_r = pltpu.roll(inv, 4, 0)
                ie = jnp.where(lo4, inv_r, inv)
                io = jnp.where(lo4, inv, inv_r)
                mid = jnp.where(lo4, a, b) * inv_r
                pair = 2 * g + pp
                ot_scr[c, 40 * pair:40 * pair + 40, :] = jnp.concatenate(
                    [re[0:8] * ie, re[8:16] * ie, mid, ro[8:16] * io, ro[16:24] * io], axis=0)
            if g == NG - 1:
                finish(c)

        def finish(c):
            o = ot_scr[c].T
            hl = (lax.broadcasted_iota(jnp.int32, (32, D), 1) * 3277) >> 16
            h1 = (hl & 1) != 0
            h2 = (hl & 2) != 0
            b4 = [o[32 * j:32 * (j + 1)] for j in range(4)]
            u = [jnp.where(h1, b4[j ^ 1], b4[j]) for j in range(4)]
            out = [jnp.where(h2, u[j ^ 2], u[j]) for j in range(4)]
            o_scr[c * 128:(c + 1) * 128, :] = jnp.concatenate(out, axis=0).astype(bf16)

        if first:
            items = [((1, 0), g) for g in range(NG)]
        else:
            items = [((c,), g) for c in range(NQT) for g in range(NG)]
        n = len(items)
        head, tail1, tail2 = (HEAD0, TAIL10, TAIL20) if first else (HEAD, TAIL1, TAIL2)
        keep = tail1 + tail2
        run(head)
        navail = max(len(dq) - keep, 0)
        ms = {}
        for i in range(n + 1):
            if i < n:
                ms[i] = {c: qk(c, items[i][1], i % 2) for c in items[i][0]}
            nd = ((i + 1) * navail) // (n + 1) - (i * navail) // (n + 1)
            if i == 0:
                run(nd, keep)
                continue
            cs, g = items[i - 1]
            groups = [(c, kt) for c in cs for kt in range(tmin(c) // 4, 3)]
            pre = [0, 0, 0]
            for q in range(nd):
                pre[((2, 1, 0) if i < n else (0, 2, 1))[q % 3]] += 1
            for gi, ((c, kt), m) in enumerate(zip(groups, pre)):
                if first and gi == 2:
                    if i == WAIT_AT:
                        for name in ("wo", "wga", "wua", "x2"):
                            copies[name].wait()
                    if 0 <= i - WAIT_AT < 4:
                        ln1_part(2, 0, i - WAIT_AT)
                run(m, keep)
                pv(c, g, kt, (i - 1) % 2, ms[i - 1][c])
        run(tail1)

        hs = {}

        def h_done(n, val):
            hs[n] = xs[0, rows_of(blk), n * 128:(n + 1) * 128].astype(f32) + val
            h_scr[blk % 2, :, n * 128:(n + 1) * 128] = hs[n]

        o_cols = _lazy_cols(lambda: o_scr[...])
        tiles = [(o_cols, lambda a, k0, k1, n=n: _dot(a, wo[k0:k1, n * 128:(n + 1) * 128]),
                  functools.partial(h_done, n)) for n in range(5)]
        for ch in _proj_chunks(tiles, *stage(0)):
            ch()
        hn = _ln(jnp.concatenate([hs[n] for n in range(5)], axis=1)).astype(bf16)
        hn_scr[...] = hn
        run(len(dq))
        for ch in gu_chunks(lambda k0, k1: hn[:, k0:k1], True):
            ch()

    @pl.when(step == 0)
    def _():
        for c in copies.values():
            c.start()

        def go(tiles):
            for ch in _proj_chunks(tiles, *stage(1)):
                ch()

        xn = []
        for b in range(2):
            copies["x%d" % b].wait()
            v = _ln(xs[0, rows_of(b), :].astype(f32)).astype(bf16)
            xn.append(lambda k0, k1, v=v: v[:, k0:k1])
        kt = [qkv_tiles(b, xn[b], "k") for b in range(2)]
        copies["wka"].wait()
        go(kt[0][:KA] + kt[1][:KA])
        copies["wkb"].wait()
        go(kt[0][KA:] + kt[1][KA:])
        copies["wq"].wait()
        go(qkv_tiles(0, xn[0], "q"))
        copies["wv"].wait()
        go(qkv_tiles(0, xn[0], "v"))
        main(True, _proj_chunks(qkv_tiles(1, xn[1], "vq"), *stage(1)))
        copies["x35"].wait()

    @pl.when(jnp.logical_or(step == 1, step == 4))
    def _():
        lnq = {t0 + 2 * part: (r + 1, part) for r, t0 in enumerate(LN_AT) for part in range(4)}
        count = [0]

        def hook(val):
            job = lnq.pop(count[0], None)
            count[0] += 1
            if job:
                xs[zw, S:S + 16, 0:128] = val[0:16].astype(bf16)
                ln1_part(jnp.minimum(step + 1 + job[0], NB - 1), job[0] % 3, job[1])

        for name, r in UNITS:
            r = int(r)
            xn = lambda k0, k1, r=r: xn_scr[r][zr, 0:T, k0:k1]
            for ch in _proj_chunks(qkv_tiles(step + 1 + r, xn, name, hook), *stage(1)):
                ch()

    @pl.when(step == 1)
    def _():
        for name in ("wg2", "wu2", "wgb", "wub", "wd", "x67"):
            copies[name].wait()

    @pl.when(jnp.logical_and(step > 0, step < NB))
    def _():
        main(False, deferred())

    @pl.when(step == NB)
    def _():
        for ch in deferred(True):
            ch()
        cp(ob, o_hbm, sems.at[0]).wait()


@jax.jit
def pallas_sequential_preLN__sliding_block__glu_gated_glu__prompt_kernel(
    A_x: jax.Array,
    A_wqkv: jax.Array,
    A_wo: jax.Array,
    B_x: jax.Array,
    B_w_gate: jax.Array,
    B_w_up: jax.Array,
    B_w_down: jax.Array,
):
    del B_x
    hbm = pl.BlockSpec(memory_space=pl.ANY)
    out = pl.pallas_call(
        _kernel,
        grid=(NB + 1,),
        in_specs=[hbm] * 6,
        out_specs=hbm,
        out_shape=jax.ShapeDtypeStruct((S, D), bf16),
        scratch_shapes=[
            pltpu.VMEM((S, D), bf16),
            pltpu.VMEM((1, S + 64, D), bf16),
            pltpu.VMEM((D, 3 * D), bf16),
            pltpu.VMEM((D, D), bf16),
            pltpu.VMEM((2 * F, D), bf16),
            pltpu.VMEM((F, D), bf16),
            pltpu.SemaphoreType.DMA((9,)),
            pltpu.VMEM((NG, S, 128), bf16),
            pltpu.VMEM((NG, S, 128), f32),
            pltpu.VMEM((S // 128, 48 * NP, 128), f32),
            pltpu.VMEM((NQT, D, 128), f32),
            pltpu.VMEM((T, D), bf16),
            pltpu.VMEM((2, T, D), f32),
            pltpu.VMEM((T, D), bf16),
            pltpu.VMEM((T, F), f32),
        ] + [pltpu.VMEM((1, 4, 384, 128), f32)] * 2
        + [pltpu.VMEM((1, T, 128), f32)] * 9
        + [pltpu.VMEM((1, T + 32, D), f32)] * 3,
        compiler_params=pltpu.CompilerParams(
            dimension_semantics=("arbitrary",),
            vmem_limit_bytes=100 * 1024 * 1024),
        name="fused_block",
    )(A_x.reshape(S, D), A_wqkv, A_wo, B_w_gate.T, B_w_up.T, B_w_down)
    return out.reshape(1, S, D)
```

```python
import functools
import math

import jax
import jax.numpy as jnp
from jax import lax
import jax.experimental.pallas as pl
import jax.experimental.pallas.tpu as pltpu

S, D, H, DH, F = 2048, 640, 32, 20, 1728
T = 256
NB = S // T
NQT = T // 128
NG = H // 4
NP = H // 2
FT = F // 128
FM = FT * 128
NEG = -1e9
EPS = 1e-5
QSCALE = (DH ** -0.5) * math.log2(math.e)
f32, bf16, u32 = jnp.float32, jnp.bfloat16, jnp.uint32

FA = 256
HEAD, TAIL1, TAIL2 = 3, 2, 2
HEAD0, TAIL10, TAIL20 = 0, 3, 4
KA = 2
WAIT_AT = 5
UNITS = ("q0", "k0", "q1", "k1", "q2", "v0", "v1", "v2", "k2")
LN_AT = (0, 10, 30)


def _ln(x):
    m = jnp.mean(x, axis=-1, keepdims=True)
    xc = x - m
    v = jnp.mean(xc * xc, axis=-1, keepdims=True)
    return xc * lax.rsqrt(v + EPS)


def _sel(mask, a, b):
    if a is None and b is None:
        return None
    if a is None:
        a = jnp.zeros_like(b)
    if b is None:
        b = jnp.zeros_like(a)
    return jnp.where(mask, a, b)


def _sigmoid(x):
    return 0.5 * jnp.tanh(0.5 * x) + 0.5


def _dot(a, b):
    return jnp.dot(a, b, preferred_element_type=f32)


def _dot_nt(a, b):
    return lax.dot_general(a, b, (((1,), (1,)), ((), ())), preferred_element_type=f32)


def _proj_chunks(tiles, put, get):
    chunks = []

    def tail(group):
        def run():
            ns = {4: 1, 2: 2}.get(len(group), 4)
            for slot, (lhs, fn, _) in enumerate(group):
                a = lhs(512, D)
                q = a.shape[0] // ns
                put(slot, jnp.concatenate(
                    [fn(a[r * q:(r + 1) * q], 512, D) for r in range(ns)], axis=0))
        return run

    def head(slot, lhs, fn, done):
        def run():
            a = lhs(0, 512)
            done(get(slot, a.shape[0]) + fn(a, 0, 512))
        return run

    for i in range(0, len(tiles), 4):
        group = tiles[i:i + 4]
        chunks.append(tail(group))
        chunks += [head(slot, *tile) for slot, tile in enumerate(group)]
    return chunks


def _lazy_cols(fn):
    cache = []

    def get(k0, k1):
        if not cache:
            cache.append(fn())
        return cache[0][:, k0:k1]
    return get


def _kernel(x_hbm, wqkv_hbm, wo_hbm, wg_hbm, wu_hbm, wd_hbm, o_hbm,
            ob, xs, wqkv, wo, wgu, wd, sems,
            q_scr, k_scr, vt_scr, ot_scr, o_scr, h_scr, hn_scr, act_scr, *bufs):
    phase = pl.program_id(0)
    s_scr, g_scr = bufs[0:2], bufs[2]
    sets, xn_scr = [bufs[3:7], bufs[7:11]], bufs[11:14]
    a_scr = xn_scr
    zw = lax.shift_right_logical(phase, 8)
    zr = lax.shift_right_logical(phase, 9)

    def stage(k):
        def put(slot, val):
            sets[k][slot][zw, 0:val.shape[0]] = val

        def get(slot, n):
            return sets[k][slot][zr, 0:n]
        return put, get

    cp = pltpu.make_async_copy
    ka = D + 128 * KA
    copies = dict(
        x0=cp(x_hbm.at[0:T], xs.at[0, 0:T], sems.at[0]),
        x1=cp(x_hbm.at[T:2 * T], xs.at[0, T:2 * T], sems.at[1]),
        wka=cp(wqkv_hbm.at[:, D:ka], wqkv.at[:, D:ka], sems.at[2]),
        wkb=cp(wqkv_hbm.at[:, ka:2 * D], wqkv.at[:, ka:2 * D], sems.at[3]),
        wq=cp(wqkv_hbm.at[:, 0:D], wqkv.at[:, 0:D], sems.at[4]),
        wv=cp(wqkv_hbm.at[:, 2 * D:3 * D], wqkv.at[:, 2 * D:3 * D], sems.at[5]),
        wo=cp(wo_hbm, wo, sems.at[6]),
        wga=cp(wg_hbm.at[0:FA], wgu.at[0:FA], sems.at[6]),
        wua=cp(wu_hbm.at[0:FA], wgu.at[FM:FM + FA], sems.at[6]),
        x2=cp(x_hbm.at[2 * T:3 * T], xs.at[0, 2 * T:3 * T], sems.at[6]),
        x35=cp(x_hbm.at[3 * T:6 * T], xs.at[0, 3 * T:6 * T], sems.at[7]),
        wg2=cp(wg_hbm.at[FM:F], wgu.at[2 * FM:2 * FM + 64], sems.at[8]),
        wu2=cp(wu_hbm.at[FM:F], wgu.at[2 * FM + 64:2 * F], sems.at[8]),
        wgb=cp(wg_hbm.at[FA:FM], wgu.at[FA:FM], sems.at[8]),
        wub=cp(wu_hbm.at[FA:FM], wgu.at[FM + FA:2 * FM], sems.at[8]),
        wd=cp(wd_hbm, wd, sems.at[8]),
        x67=cp(x_hbm.at[6 * T:8 * T], xs.at[0, 6 * T:8 * T], sems.at[8]),
    )

    def rows_of(b, n=T):
        return pl.ds(b * T if isinstance(b, int) else pl.multiple_of(b * T, T), n)

    def ocopy(b):
        return cp(ob.at[rows_of(b)], o_hbm.at[rows_of(b)], sems.at[0])

    def ocopy_last(n):
        rows, cols = rows_of(NB - 1), pl.ds(n * 128, 128)
        return cp(ob.at[rows, cols], o_hbm.at[rows, cols], sems.at[0])

    lo4 = lax.broadcasted_iota(jnp.int32, (8, 128), 0) < 4

    def qkv_tiles(b, xn, which, hook=None, cs=tuple(range(NQT))):
        got = {}
        r0, nr = cs[0] * 128, len(cs) * 128
        lane = lax.broadcasted_iota(jnp.int32, (nr, 128), 1)

        def done(key, val):
            name, n = key
            if hook:
                hook(val)
            if name == "v":
                for c in cs:
                    vt = val[c * 128 - r0:(c + 1) * 128 - r0, :].T
                    for i in range(16):
                        p, e = divmod(16 * n + i, 5)
                        piece = vt[8 * i:8 * i + 8]
                        kt = b * NQT + c
                        if e == 2:
                            vt_scr[kt, 48 * p + 16:48 * p + 24, :] = jnp.where(lo4, piece, 1.0)
                            vt_scr[kt, 48 * p + 24:48 * p + 32, :] = jnp.where(lo4, 1.0, piece)
                        else:
                            o = 48 * p + 8 * (e if e < 2 else e + 1)
                            vt_scr[kt, o:o + 8, :] = piece
                return
            if name == "q":
                val = val * QSCALE
            got[key] = val
            for g in range(NG):
                lo = 80 * g
                t0, t1 = lo // 128, (lo + 79) // 128
                if t1 != n:
                    continue
                tile = val if t0 == t1 else jnp.where(lane >= lo % 128, got[(name, t0)], val)
                if name == "q":
                    q_scr.at[g, rows_of(b)][r0:r0 + nr, :] = tile.astype(bf16)
                else:
                    k_scr.at[g, rows_of(b)][r0:r0 + nr, :] = tile

        base = {"q": 0, "k": D, "v": 2 * D}
        tiles = []
        for name in which:
            for n in range(5):
                c0 = base[name] + 128 * n
                tiles.append((lambda k0, k1: xn(k0, k1)[r0:r0 + nr],
                              lambda a, k0, k1, c0=c0: _dot(a, wqkv[k0:k1, c0:c0 + 128]),
                              functools.partial(done, (name, n))))
        return tiles

    def ln1_part(b, r, part):
        rows = slice(part * T // 4, (part + 1) * T // 4)
        xn_scr[r][zw, rows, :] = _ln(xs.at[zr, rows_of(b)][rows, :].astype(f32))

    def gu_chunks(hn, head):
        def done(key, val):
            name, f = key
            if name == "g":
                g_scr[zw] = _sigmoid(val)
            elif name == "u":
                act_scr[:, f * 128:(f + 1) * 128] = g_scr[zr] * val
            else:
                act_scr[:, FM:F] = (_sigmoid(val) * pltpu.roll(val, 64, 1))[:, 0:64]

        tiles = []
        for f in range(FT):
            for name, r0 in (("g", f * 128), ("u", FM + f * 128)):
                tiles.append((hn, lambda a, k0, k1, r0=r0: _dot_nt(a, wgu[r0:r0 + 128, k0:k1]),
                              functools.partial(done, (name, f))))
        tiles.append((hn, lambda a, k0, k1: _dot_nt(a, wgu[2 * FM:2 * F, k0:k1]),
                      functools.partial(done, ("gu", FT))))
        return _proj_chunks(tiles[:FA // 64] if head else tiles[FA // 64:], *stage(0))

    def deferred(step, last=False):
        par = (step + 1) % 2

        def d_chunk(n0, n1, k0, k1, nsplit=1, then=None):
            def run():
                cols = slice(n0 * 128, n1 * 128)
                q = T // nsplit
                for r in range(nsplit):
                    rows = slice(r * q, (r + 1) * q)
                    y = h_scr[par, rows, cols] + _dot(act_scr[rows, k0:k1], wd[k0:k1, cols])
                    if k1 == F:
                        ob.at[rows_of(step - 1)][rows, cols] = y.astype(bf16)
                    else:
                        h_scr[par, rows, cols] = y
                if then:
                    then().start()
            return run

        early = [d_chunk(0, 2, 0, 256), d_chunk(2, 4, 0, 256), d_chunk(4, 5, 0, 256, 2)]
        ks = ((256, 768), (768, 1280), (1280, F))
        if last:
            late = [d_chunk(n, n + 1, k0, k1,
                            then=functools.partial(ocopy_last, n) if k1 == F else None)
                    for n in range(5) for k0, k1 in ks]
        else:
            late = [d_chunk(n, n + 1, k0, k1,
                            then=(lambda: ocopy(step - 1)) if (k1 == F and n == 4) else None)
                    for k0, k1 in ks for n in range(5)]
        return early + gu_chunks(_lazy_cols(lambda: hn_scr[...]), False) + late

    def main(step, dq):
        first = isinstance(step, int)
        blk = step
        lane16 = lax.broadcasted_iota(jnp.int32, (16, 128), 1)
        lane32 = lax.broadcasted_iota(jnp.int32, (32, 128), 1)
        m_s1 = (lane32 & 32) != 0
        m_s2 = (lane32 & 64) != 0
        tri_first = lax.broadcasted_iota(jnp.int32, (32, 128), 0) > (lane32 & 31)
        kv = k_scr if first else k_scr.at[:, rows_of(step - 1, 2 * T)]
        koff = -T if first else 0
        qv = q_scr.at[:, rows_of(blk)]
        kt0 = blk * NQT
        tmin = lambda c: max(0, 8 - 4 * c) if first else 0
        soff = lambda c: -8 if first and c == 0 else 0

        def run(n, keep=0):
            for _ in range(n):
                if len(dq) > keep:
                    dq.pop(0)()

        def qk(c, g, buf):
            ms = {}
            for j in (3, 2, 1, 0):
                t0, t1 = max(j, tmin(c)), j + 9
                rows = (t1 - t0) * 32
                start = koff + c * 128 + t0 * 32
                qb = pltpu.bitcast(qv[g, c * 128 + j * 32:c * 128 + (j + 1) * 32, :], u32)
                slots = []
                for s in range(4):
                    lo = (80 * g + 20 * (s ^ j)) % 128
                    slots.append(jnp.where(((lane16 - lo) & 127) < DH, qb, jnp.zeros_like(qb)))
                qm = pltpu.bitcast(jnp.concatenate(slots, axis=0), bf16)
                st = _dot_nt(kv[g, start:start + rows, :], qm)
                parts = []
                if t0 == j:
                    parts.append(jnp.where(tri_first, st[0:32], NEG))
                    parts.append(st[32:rows - 32])
                elif rows > 32:
                    parts.append(st[0:rows - 32])
                parts.append(jnp.where(tri_first, NEG, st[rows - 32:rows]))
                st = jnp.concatenate(parts, axis=0)
                ms[j] = jnp.max(st, axis=0, keepdims=True)
                s_scr[buf][zw, j, (t0 + soff(c)) * 32:(t1 + soff(c)) * 32, :] = st
            return ms

        def probs(c, kt, sbuf, ms):
            ph = [[] for _ in range(4)]
            for t in range(4 * kt, 4 * kt + 4):
                ts = t + soff(c)
                p = [jnp.exp2(s_scr[sbuf][zr, j, ts * 32:(ts + 1) * 32, :] - ms[j])
                     if j <= t <= j + 8 else None for j in range(4)]
                u = [_sel(m_s1, p[j ^ 1], p[j]) for j in range(4)]
                for h in range(4):
                    ph[h].append(_sel(m_s2, u[h ^ 2], u[h]))
            return [jnp.concatenate(ph[h], axis=0).astype(bf16) for h in range(4)]

        def pv(c, g, kt, sbuf, ms):
            ps = probs(c, kt, sbuf, ms)
            res = []
            for h in range(4):
                r0 = 48 * (2 * g + h // 2) + 24 * (h % 2)
                r = _dot(vt_scr[kt0 + c - 2 + kt, r0:r0 + 24, :], ps[h])
                if kt > tmin(c) // 4:
                    r = r + a_scr[kt - 1][zr, T:T + 24, h * 128:(h + 1) * 128]
                if kt < 2:
                    a_scr[kt][zw, T:T + 24, h * 128:(h + 1) * 128] = r
                res.append(r)
            if kt < 2:
                return
            for pp in range(2):
                re, ro = res[2 * pp], res[2 * pp + 1]
                a, b = re[16:24], ro[0:8]
                l = jnp.where(lo4, b, a)
                inv = pl.reciprocal(l, approx=True)
                inv = inv * (2.0 - l * inv)
                inv_r = pltpu.roll(inv, 4, 0)
                ie = jnp.where(lo4, inv_r, inv)
                io = jnp.where(lo4, inv, inv_r)
                mid = jnp.where(lo4, a, b) * inv_r
                pair = 2 * g + pp
                ot_scr[c, 40 * pair:40 * pair + 40, :] = jnp.concatenate(
                    [re[0:8] * ie, re[8:16] * ie, mid, ro[8:16] * io, ro[16:24] * io], axis=0)
            if g == NG - 1:
                finish(c)

        def finish(c):
            o = ot_scr[c].T
            hl = (lax.broadcasted_iota(jnp.int32, (32, D), 1) * 3277) >> 16
            h1 = (hl & 1) != 0
            h2 = (hl & 2) != 0
            b4 = [o[32 * j:32 * (j + 1)] for j in range(4)]
            u = [jnp.where(h1, b4[j ^ 1], b4[j]) for j in range(4)]
            out = [jnp.where(h2, u[j ^ 2], u[j]) for j in range(4)]
            o_scr[c * 128:(c + 1) * 128, :] = jnp.concatenate(out, axis=0).astype(bf16)

        if first:
            items = [((1, 0), g) for g in range(NG)]
        else:
            items = [((c,), g) for c in range(NQT) for g in range(NG)]
        n = len(items)
        head, tail1, tail2 = (HEAD0, TAIL10, TAIL20) if first else (HEAD, TAIL1, TAIL2)
        keep = tail1 + tail2
        run(head)
        navail = max(len(dq) - keep, 0)
        ms = {}
        for i in range(n + 1):
            if i < n:
                ms[i] = {c: qk(c, items[i][1], i % 2) for c in items[i][0]}
            nd = ((i + 1) * navail) // (n + 1) - (i * navail) // (n + 1)
            if i == 0:
                run(nd, keep)
                continue
            cs, g = items[i - 1]
            groups = [(c, kt) for c in cs for kt in range(tmin(c) // 4, 3)]
            pre = [0, 0, 0]
            for q in range(nd):
                pre[((2, 1, 0) if i < n else (0, 2, 1))[q % 3]] += 1
            for gi, ((c, kt), m) in enumerate(zip(groups, pre)):
                if first and gi == 2:
                    if i == WAIT_AT:
                        for name in ("wo", "wga", "wua", "x2"):
                            copies[name].wait()
                    if 0 <= i - WAIT_AT < 4:
                        ln1_part(2, 0, i - WAIT_AT)
                run(m, keep)
                pv(c, g, kt, (i - 1) % 2, ms[i - 1][c])
        run(tail1)

        hs = {}

        def h_done(n, val):
            hs[n] = xs[0, rows_of(blk), n * 128:(n + 1) * 128].astype(f32) + val
            h_scr[blk % 2, :, n * 128:(n + 1) * 128] = hs[n]

        o_cols = _lazy_cols(lambda: o_scr[...])
        tiles = [(o_cols, lambda a, k0, k1, n=n: _dot(a, wo[k0:k1, n * 128:(n + 1) * 128]),
                  functools.partial(h_done, n)) for n in range(5)]
        for ch in _proj_chunks(tiles, *stage(0)):
            ch()
        hn = _ln(jnp.concatenate([hs[n] for n in range(5)], axis=1)).astype(bf16)
        hn_scr[...] = hn
        run(len(dq))
        for ch in gu_chunks(lambda k0, k1: hn[:, k0:k1], True):
            ch()

    @pl.when(phase == 0)
    def _():
        for c in copies.values():
            c.start()

        def go(tiles):
            for ch in _proj_chunks(tiles, *stage(1)):
                ch()

        xn = []
        for b in range(2):
            copies["x%d" % b].wait()
            v = _ln(xs[0, rows_of(b), :].astype(f32)).astype(bf16)
            xn.append(lambda k0, k1, v=v: v[:, k0:k1])
        kt = [qkv_tiles(b, xn[b], "k") for b in range(2)]
        copies["wka"].wait()
        go(kt[0][:KA] + kt[1][:KA])
        copies["wkb"].wait()
        go(kt[0][KA:] + kt[1][KA:])
        copies["wq"].wait()
        go(qkv_tiles(0, xn[0], "q"))
        copies["wv"].wait()
        go(qkv_tiles(0, xn[0], "v"))
        half = [t for name in "vq" for c in range(NQT) for t in qkv_tiles(1, xn[1], name, cs=(c,))]
        main(0, _proj_chunks(half, *stage(1)))
        copies["x35"].wait()

    def qkv3(step):
        lnq = {t0 + 2 * part: (r + 1, part) for r, t0 in enumerate(LN_AT) for part in range(4)}
        count = [0]

        def hook(val):
            job = lnq.pop(count[0], None)
            count[0] += 1
            if job:
                xs[zw, S:S + 16, 0:128] = val[0:16].astype(bf16)
                ln1_part(jnp.minimum(step + 1 + job[0], NB - 1), job[0] % 3, job[1])

        for name, r in UNITS:
            r = int(r)
            xn = lambda k0, k1, r=r: xn_scr[r][zr, 0:T, k0:k1]
            for ch in _proj_chunks(qkv_tiles(step + 1 + r, xn, name, hook), *stage(1)):
                ch()

    @pl.when(phase == 1)
    def _():
        def body(step, carry):
            @pl.when(jnp.logical_or(step == 1, step == 4))
            def _():
                qkv3(step)

                @pl.when(step == 1)
                def _():
                    for name in ("wg2", "wu2", "wgb", "wub", "wd", "x67"):
                        copies[name].wait()

            main(step, deferred(step))
            return carry

        lax.fori_loop(1, NB, body, 0)

    @pl.when(phase == 2)
    def _():
        for ch in deferred(NB, True):
            ch()
        cp(ob, o_hbm, sems.at[0]).wait()


@jax.jit
def pallas_sequential_preLN__sliding_block__glu_gated_glu__prompt_kernel(
    A_x: jax.Array,
    A_wqkv: jax.Array,
    A_wo: jax.Array,
    B_x: jax.Array,
    B_w_gate: jax.Array,
    B_w_up: jax.Array,
    B_w_down: jax.Array,
):
    del B_x
    hbm = pl.BlockSpec(memory_space=pl.ANY)
    out = pl.pallas_call(
        _kernel,
        grid=(3,),
        in_specs=[hbm] * 6,
        out_specs=hbm,
        out_shape=jax.ShapeDtypeStruct((S, D), bf16),
        scratch_shapes=[
            pltpu.VMEM((S, D), bf16),
            pltpu.VMEM((1, S + 64, D), bf16),
            pltpu.VMEM((D, 3 * D), bf16),
            pltpu.VMEM((D, D), bf16),
            pltpu.VMEM((2 * F, D), bf16),
            pltpu.VMEM((F, D), bf16),
            pltpu.SemaphoreType.DMA((9,)),
            pltpu.VMEM((NG, S, 128), bf16),
            pltpu.VMEM((NG, S, 128), f32),
            pltpu.VMEM((S // 128, 48 * NP, 128), f32),
            pltpu.VMEM((NQT, D, 128), f32),
            pltpu.VMEM((T, D), bf16),
            pltpu.VMEM((2, T, D), f32),
            pltpu.VMEM((T, D), bf16),
            pltpu.VMEM((T, F), f32),
        ] + [pltpu.VMEM((1, 4, 384, 128), f32)] * 2
        + [pltpu.VMEM((1, T, 128), f32)] * 9
        + [pltpu.VMEM((1, T + 32, D), f32)] * 3,
        compiler_params=pltpu.CompilerParams(
            dimension_semantics=("arbitrary",),
            vmem_limit_bytes=100 * 1024 * 1024),
        name="fused_block",
    )(A_x.reshape(S, D), A_wqkv, A_wo, B_w_gate.T, B_w_up.T, B_w_down)
    return out.reshape(1, S, D)
```

```python
import functools
import math

import jax
import jax.numpy as jnp
from jax import lax
import jax.experimental.pallas as pl
import jax.experimental.pallas.tpu as pltpu

S, D, H, DH, F = 2048, 640, 32, 20, 1728
T = 256
NB = S // T
NQT = T // 128
NG = H // 4
NP = H // 2
FT = F // 128
FM = FT * 128
NEG = -1e9
EPS = 1e-5
QSCALE = (DH ** -0.5) * math.log2(math.e)
f32, bf16 = jnp.float32, jnp.bfloat16

FA = 256
HEAD, TAIL1, TAIL2 = 3, 2, 2
HEAD0, TAIL10, TAIL20 = 0, 3, 4
KA = 2
WAIT_AT = 5
UNITS = ("q0", "k0", "q1", "k1", "q2", "v0", "v1", "v2", "k2")
LN_AT = (1, 9, 31)


def _ln(x):
    m = jnp.mean(x, axis=-1, keepdims=True)
    xc = x - m
    v = jnp.mean(xc * xc, axis=-1, keepdims=True)
    return xc * lax.rsqrt(v + EPS)


def _sel(mask, a, b):
    if a is None and b is None:
        return None
    if a is None:
        a = jnp.zeros_like(b)
    if b is None:
        b = jnp.zeros_like(a)
    return jnp.where(mask, a, b)


def _sigmoid(x):
    return 0.5 * jnp.tanh(0.5 * x) + 0.5


def _dot(a, b):
    return jnp.dot(a, b, preferred_element_type=f32)


def _dot_nt(a, b):
    return lax.dot_general(a, b, (((1,), (1,)), ((), ())), preferred_element_type=f32)


def _proj_chunks(tiles, put, get):
    chunks = []

    def tail(group):
        def run():
            ns = {4: 1, 2: 2}.get(len(group), 4)
            for slot, (lhs, fn, _) in enumerate(group):
                a = lhs(512, D)
                q = a.shape[0] // ns
                put(slot, jnp.concatenate(
                    [fn(a[r * q:(r + 1) * q], 512, D) for r in range(ns)], axis=0))
        return run

    def head(slot, lhs, fn, done):
        def run():
            a = lhs(0, 512)
            done(get(slot, a.shape[0]) + fn(a, 0, 512))
        return run

    for i in range(0, len(tiles), 4):
        group = tiles[i:i + 4]
        chunks.append(tail(group))
        chunks += [head(slot, *tile) for slot, tile in enumerate(group)]
    return chunks


def _lazy_cols(fn):
    cache = []

    def get(k0, k1):
        if not cache:
            cache.append(fn())
        return cache[0][:, k0:k1]
    return get


def _kernel(x_hbm, wqkv_hbm, wo_hbm, wg_hbm, wu_hbm, wd_hbm, o_hbm,
            ob, xs, wqkv, wo, wgu, wd, sems,
            q_scr, k_scr, vt_scr, ot_scr, o_scr, h_scr, hn_scr, act_scr, *bufs):
    phase = pl.program_id(0)
    s_scr, g_scr = bufs[0:2], bufs[2]
    sets, xn_scr = [bufs[3:7], bufs[7:11]], bufs[11:14]
    a_scr = xn_scr
    zw = lax.shift_right_logical(phase, 8)
    zr = lax.shift_right_logical(phase, 9)

    def stage(k):
        def put(slot, val):
            sets[k][slot][zw, 0:val.shape[0]] = val

        def get(slot, n):
            return sets[k][slot][zr, 0:n]
        return put, get

    cp = pltpu.make_async_copy
    ka = D + 128 * KA
    copies = dict(
        x0=cp(x_hbm.at[0:T], xs.at[0, 0:T], sems.at[0]),
        x1=cp(x_hbm.at[T:2 * T], xs.at[0, T:2 * T], sems.at[1]),
        wka=cp(wqkv_hbm.at[:, D:ka], wqkv.at[:, D:ka], sems.at[2]),
        wkb=cp(wqkv_hbm.at[:, ka:2 * D], wqkv.at[:, ka:2 * D], sems.at[3]),
        wq=cp(wqkv_hbm.at[:, 0:D], wqkv.at[:, 0:D], sems.at[4]),
        wv=cp(wqkv_hbm.at[:, 2 * D:3 * D], wqkv.at[:, 2 * D:3 * D], sems.at[5]),
        wo=cp(wo_hbm, wo, sems.at[6]),
        wga=cp(wg_hbm.at[0:FA], wgu.at[0:FA], sems.at[6]),
        wua=cp(wu_hbm.at[0:FA], wgu.at[FM:FM + FA], sems.at[6]),
        x2=cp(x_hbm.at[2 * T:3 * T], xs.at[0, 2 * T:3 * T], sems.at[6]),
        x35=cp(x_hbm.at[3 * T:6 * T], xs.at[0, 3 * T:6 * T], sems.at[7]),
        wg2=cp(wg_hbm.at[FM:F], wgu.at[2 * FM:2 * FM + 64], sems.at[8]),
        wu2=cp(wu_hbm.at[FM:F], wgu.at[2 * FM + 64:2 * F], sems.at[8]),
        wgb=cp(wg_hbm.at[FA:FM], wgu.at[FA:FM], sems.at[8]),
        wub=cp(wu_hbm.at[FA:FM], wgu.at[FM + FA:2 * FM], sems.at[8]),
        wd=cp(wd_hbm, wd, sems.at[8]),
        x67=cp(x_hbm.at[6 * T:8 * T], xs.at[0, 6 * T:8 * T], sems.at[8]),
    )

    def rows_of(b, n=T):
        return pl.ds(b * T if isinstance(b, int) else pl.multiple_of(b * T, T), n)

    def ocopy(b):
        return cp(ob.at[rows_of(b)], o_hbm.at[rows_of(b)], sems.at[0])

    def ocopy_last(n):
        rows, cols = rows_of(NB - 1), pl.ds(n * 128, 128)
        return cp(ob.at[rows, cols], o_hbm.at[rows, cols], sems.at[0])

    lo4 = lax.broadcasted_iota(jnp.int32, (8, 128), 0) < 4

    def qkv_tiles(b, xn, which, hook=None, cs=tuple(range(NQT))):
        got = {}
        r0, nr = cs[0] * 128, len(cs) * 128
        lane = lax.broadcasted_iota(jnp.int32, (nr, 128), 1)

        def done(key, val):
            name, n = key
            if hook:
                hook(val)
            if name == "v":
                for c in cs:
                    vt = val[c * 128 - r0:(c + 1) * 128 - r0, :].T
                    for i in range(16):
                        p, e = divmod(16 * n + i, 5)
                        piece = vt[8 * i:8 * i + 8]
                        kt = b * NQT + c
                        if e == 2:
                            vt_scr[kt, 48 * p + 16:48 * p + 24, :] = jnp.where(lo4, piece, 1.0)
                            vt_scr[kt, 48 * p + 24:48 * p + 32, :] = jnp.where(lo4, 1.0, piece)
                        else:
                            o = 48 * p + 8 * (e if e < 2 else e + 1)
                            vt_scr[kt, o:o + 8, :] = piece
                return
            if name == "q":
                val = val * QSCALE
            got[key] = val
            for g in range(NG):
                lo = 80 * g
                t0, t1 = lo // 128, (lo + 79) // 128
                if t1 != n:
                    continue
                tile = val if t0 == t1 else jnp.where(lane >= lo % 128, got[(name, t0)], val)
                if name == "q":
                    q_scr.at[g, rows_of(b)][r0:r0 + nr, :] = tile
                else:
                    k_scr.at[g, rows_of(b)][r0:r0 + nr, :] = tile

        base = {"q": 0, "k": D, "v": 2 * D}
        tiles = []
        for name in which:
            for n in range(5):
                c0 = base[name] + 128 * n
                tiles.append((lambda k0, k1: xn(k0, k1)[r0:r0 + nr],
                              lambda a, k0, k1, c0=c0: _dot(a, wqkv[k0:k1, c0:c0 + 128]),
                              functools.partial(done, (name, n))))
        return tiles

    def ln1_part(b, r, part):
        rows = slice(part * T // 4, (part + 1) * T // 4)
        xn_scr[r][zw, rows, :] = _ln(xs.at[zr, rows_of(b)][rows, :].astype(f32))

    def gu_chunks(hn, head):
        def done(key, val):
            name, f = key
            if name == "g":
                g_scr[zw] = _sigmoid(val)
            elif name == "u":
                act_scr[:, f * 128:(f + 1) * 128] = g_scr[zr] * val
            else:
                act_scr[:, FM:F] = (_sigmoid(val) * pltpu.roll(val, 64, 1))[:, 0:64]

        tiles = []
        for f in range(FT):
            for name, r0 in (("g", f * 128), ("u", FM + f * 128)):
                tiles.append((hn, lambda a, k0, k1, r0=r0: _dot_nt(a, wgu[r0:r0 + 128, k0:k1]),
                              functools.partial(done, (name, f))))
        tiles.append((hn, lambda a, k0, k1: _dot_nt(a, wgu[2 * FM:2 * F, k0:k1]),
                      functools.partial(done, ("gu", FT))))
        return _proj_chunks(tiles[:FA // 64] if head else tiles[FA // 64:], *stage(0))

    def deferred(step, last=False):
        par = (step + 1) % 2

        def d_chunk(n0, n1, k0, k1, nsplit=1, then=None):
            def run():
                cols = slice(n0 * 128, n1 * 128)
                q = T // nsplit
                for r in range(nsplit):
                    rows = slice(r * q, (r + 1) * q)
                    y = h_scr[par, rows, cols] + _dot(act_scr[rows, k0:k1], wd[k0:k1, cols])
                    if k1 == F:
                        ob.at[rows_of(step - 1)][rows, cols] = y.astype(bf16)
                    else:
                        h_scr[par, rows, cols] = y
                if then:
                    then().start()
            return run

        early = [d_chunk(0, 2, 0, 256), d_chunk(2, 4, 0, 256), d_chunk(4, 5, 0, 256, 2)]
        ks = ((256, 768), (768, 1280), (1280, F))
        if last:
            late = [d_chunk(n, n + 1, k0, k1,
                            then=functools.partial(ocopy_last, n) if k1 == F else None)
                    for n in range(5) for k0, k1 in ks]
        else:
            late = [d_chunk(n, n + 1, k0, k1,
                            then=(lambda: ocopy(step - 1)) if (k1 == F and n == 4) else None)
                    for k0, k1 in ks for n in range(5)]
        return early + gu_chunks(_lazy_cols(lambda: hn_scr[...]), False) + late

    def main(step, dq):
        first = isinstance(step, int)
        blk = step
        lane32 = lax.broadcasted_iota(jnp.int32, (32, 128), 1)
        m_s1 = (lane32 & 32) != 0
        m_s2 = (lane32 & 64) != 0
        tri_first = lax.broadcasted_iota(jnp.int32, (32, 128), 0) > (lane32 & 31)
        kv = k_scr if first else k_scr.at[:, rows_of(step - 1, 2 * T)]
        koff = -T if first else 0
        qv = q_scr.at[:, rows_of(blk)]
        kt0 = blk * NQT
        tmin = lambda c: max(0, 8 - 4 * c) if first else 0
        soff = lambda c: -8 if first and c == 0 else 0

        def run(n, keep=0):
            for _ in range(n):
                if len(dq) > keep:
                    dq.pop(0)()

        def qk(c, g, buf):
            ms = {}
            for j in (3, 2, 1, 0):
                t0, t1 = max(j, tmin(c)), j + 9
                rows = (t1 - t0) * 32
                start = koff + c * 128 + t0 * 32
                qb = qv[g, c * 128 + j * 32:c * 128 + (j + 1) * 32, :]
                slots = []
                for s in range(4):
                    lo = (80 * g + 20 * (s ^ j)) % 128
                    slots.append(jnp.where(((lane32 - lo) & 127) < DH, qb, 0.0))
                qm = jnp.concatenate(slots, axis=0).astype(bf16)
                st = _dot_nt(kv[g, start:start + rows, :], qm)
                parts = []
                if t0 == j:
                    parts.append(jnp.where(tri_first, st[0:32], NEG))
                    parts.append(st[32:rows - 32])
                elif rows > 32:
                    parts.append(st[0:rows - 32])
                parts.append(jnp.where(tri_first, NEG, st[rows - 32:rows]))
                st = jnp.concatenate(parts, axis=0)
                ms[j] = jnp.max(st, axis=0, keepdims=True)
                s_scr[buf][zw, j, (t0 + soff(c)) * 32:(t1 + soff(c)) * 32, :] = st
            return ms

        def probs(c, kt, sbuf, ms):
            ph = [[] for _ in range(4)]
            for t in range(4 * kt, 4 * kt + 4):
                ts = t + soff(c)
                p = [jnp.exp2(s_scr[sbuf][zr, j, ts * 32:(ts + 1) * 32, :] - ms[j])
                     if j <= t <= j + 8 else None for j in range(4)]
                u = [_sel(m_s1, p[j ^ 1], p[j]) for j in range(4)]
                for h in range(4):
                    ph[h].append(_sel(m_s2, u[h ^ 2], u[h]))
            return [jnp.concatenate(ph[h], axis=0).astype(bf16) for h in range(4)]

        def pv(c, g, kt, sbuf, ms):
            ps = probs(c, kt, sbuf, ms)
            res = []
            for h in range(4):
                r0 = 48 * (2 * g + h // 2) + 24 * (h % 2)
                r = _dot(vt_scr[kt0 + c - 2 + kt, r0:r0 + 24, :], ps[h])
                if kt > tmin(c) // 4:
                    r = r + a_scr[kt - 1][zr, T:T + 24, h * 128:(h + 1) * 128]
                if kt < 2:
                    a_scr[kt][zw, T:T + 24, h * 128:(h + 1) * 128] = r
                res.append(r)
            if kt < 2:
                return
            for pp in range(2):
                re, ro = res[2 * pp], res[2 * pp + 1]
                a, b = re[16:24], ro[0:8]
                l = jnp.where(lo4, b, a)
                inv = pl.reciprocal(l, approx=True)
                inv = inv * (2.0 - l * inv)
                inv_r = pltpu.roll(inv, 4, 0)
                ie = jnp.where(lo4, inv_r, inv)
                io = jnp.where(lo4, inv, inv_r)
                mid = jnp.where(lo4, a, b) * inv_r
                pair = 2 * g + pp
                ot_scr[c, 40 * pair:40 * pair + 40, :] = jnp.concatenate(
                    [re[0:8] * ie, re[8:16] * ie, mid, ro[8:16] * io, ro[16:24] * io], axis=0)
            if g == NG - 1:
                finish(c)

        def finish(c):
            o = ot_scr[c].T
            hl = (lax.broadcasted_iota(jnp.int32, (32, D), 1) * 3277) >> 16
            h1 = (hl & 1) != 0
            h2 = (hl & 2) != 0
            b4 = [o[32 * j:32 * (j + 1)] for j in range(4)]
            u = [jnp.where(h1, b4[j ^ 1], b4[j]) for j in range(4)]
            out = [jnp.where(h2, u[j ^ 2], u[j]) for j in range(4)]
            o_scr[c * 128:(c + 1) * 128, :] = jnp.concatenate(out, axis=0).astype(bf16)

        if first:
            items = [((1, 0), g) for g in range(NG)]
        else:
            items = [((c,), g) for c in range(NQT) for g in range(NG)]
        n = len(items)
        head, tail1, tail2 = (HEAD0, TAIL10, TAIL20) if first else (HEAD, TAIL1, TAIL2)
        keep = tail1 + tail2
        run(head)
        navail = max(len(dq) - keep, 0)
        ms = {}
        for i in range(n + 1):
            if i < n:
                ms[i] = {c: qk(c, items[i][1], i % 2) for c in items[i][0]}
            nd = ((i + 1) * navail) // (n + 1) - (i * navail) // (n + 1)
            if i == 0:
                run(nd, keep)
                continue
            cs, g = items[i - 1]
            groups = [(c, kt) for c in cs for kt in range(tmin(c) // 4, 3)]
            pre = [0, 0, 0]
            for q in range(nd):
                pre[((2, 1, 0) if i < n else (0, 2, 1))[q % 3]] += 1
            for gi, ((c, kt), m) in enumerate(zip(groups, pre)):
                if first and gi == 2:
                    if i == WAIT_AT:
                        for name in ("wo", "wga", "wua", "x2"):
                            copies[name].wait()
                    if 0 <= i - WAIT_AT < 4:
                        ln1_part(2, 0, i - WAIT_AT)
                run(m, keep)
                pv(c, g, kt, (i - 1) % 2, ms[i - 1][c])
        run(tail1)

        hs = {}

        def h_done(n, val):
            hs[n] = xs[0, rows_of(blk), n * 128:(n + 1) * 128].astype(f32) + val
            h_scr[blk % 2, :, n * 128:(n + 1) * 128] = hs[n]

        o_cols = _lazy_cols(lambda: o_scr[...])
        tiles = [(o_cols, lambda a, k0, k1, n=n: _dot(a, wo[k0:k1, n * 128:(n + 1) * 128]),
                  functools.partial(h_done, n)) for n in range(5)]
        for ch in _proj_chunks(tiles, *stage(0)):
            ch()
        hn = _ln(jnp.concatenate([hs[n] for n in range(5)], axis=1)).astype(bf16)
        hn_scr[...] = hn
        run(len(dq))
        for ch in gu_chunks(lambda k0, k1: hn[:, k0:k1], True):
            ch()

    @pl.when(phase == 0)
    def _():
        for c in copies.values():
            c.start()

        def go(tiles):
            for ch in _proj_chunks(tiles, *stage(1)):
                ch()

        xn = []
        for b in range(2):
            copies["x%d" % b].wait()
            v = _ln(xs[0, rows_of(b), :].astype(f32)).astype(bf16)
            xn.append(lambda k0, k1, v=v: v[:, k0:k1])
        kt = [qkv_tiles(b, xn[b], "k") for b in range(2)]
        copies["wka"].wait()
        go(kt[0][:KA] + kt[1][:KA])
        copies["wkb"].wait()
        go(kt[0][KA:] + kt[1][KA:])
        copies["wq"].wait()
        go(qkv_tiles(0, xn[0], "q"))
        copies["wv"].wait()
        go(qkv_tiles(0, xn[0], "v"))
        half = [t for name in "vq" for c in range(NQT) for t in qkv_tiles(1, xn[1], name, cs=(c,))]
        main(0, _proj_chunks(half, *stage(1)))
        copies["x35"].wait()

    def qkv3(step):
        lnq = {t0 + 2 * part: (r + 1, part) for r, t0 in enumerate(LN_AT) for part in range(4)}
        count = [0]

        def hook(val):
            job = lnq.pop(count[0], None)
            count[0] += 1
            if job:
                xs[zw, S:S + 16, 0:128] = val[0:16].astype(bf16)
                ln1_part(jnp.minimum(step + 1 + job[0], NB - 1), job[0] % 3, job[1])

        for name, r in UNITS:
            r = int(r)
            xn = lambda k0, k1, r=r: xn_scr[r][zr, 0:T, k0:k1]
            for ch in _proj_chunks(qkv_tiles(step + 1 + r, xn, name, hook), *stage(1)):
                ch()

    @pl.when(phase == 1)
    def _():
        def body(step, carry):
            @pl.when(jnp.logical_or(step == 1, step == 4))
            def _():
                qkv3(step)

                @pl.when(step == 1)
                def _():
                    for name in ("wg2", "wu2", "wgb", "wub", "wd", "x67"):
                        copies[name].wait()

            main(step, deferred(step))
            return carry

        lax.fori_loop(1, NB, body, 0)

    @pl.when(phase == 2)
    def _():
        for ch in deferred(NB, True):
            ch()
        cp(ob, o_hbm, sems.at[0]).wait()


@jax.jit
def pallas_sequential_preLN__sliding_block__glu_gated_glu__prompt_kernel(
    A_x: jax.Array,
    A_wqkv: jax.Array,
    A_wo: jax.Array,
    B_x: jax.Array,
    B_w_gate: jax.Array,
    B_w_up: jax.Array,
    B_w_down: jax.Array,
):
    del B_x
    hbm = pl.BlockSpec(memory_space=pl.ANY)
    out = pl.pallas_call(
        _kernel,
        grid=(3,),
        in_specs=[hbm] * 6,
        out_specs=hbm,
        out_shape=jax.ShapeDtypeStruct((S, D), bf16),
        scratch_shapes=[
            pltpu.VMEM((S, D), bf16),
            pltpu.VMEM((1, S + 64, D), bf16),
            pltpu.VMEM((D, 3 * D), bf16),
            pltpu.VMEM((D, D), bf16),
            pltpu.VMEM((2 * F, D), bf16),
            pltpu.VMEM((F, D), bf16),
            pltpu.SemaphoreType.DMA((9,)),
            pltpu.VMEM((NG, S, 128), f32),
            pltpu.VMEM((NG, S, 128), f32),
            pltpu.VMEM((S // 128, 48 * NP, 128), f32),
            pltpu.VMEM((NQT, D, 128), f32),
            pltpu.VMEM((T, D), bf16),
            pltpu.VMEM((2, T, D), f32),
            pltpu.VMEM((T, D), bf16),
            pltpu.VMEM((T, F), f32),
        ] + [pltpu.VMEM((1, 4, 384, 128), f32)] * 2
        + [pltpu.VMEM((1, T, 128), f32)] * 9
        + [pltpu.VMEM((1, T + 32, D), f32)] * 3,
        compiler_params=pltpu.CompilerParams(
            dimension_semantics=("arbitrary",),
            vmem_limit_bytes=100 * 1024 * 1024),
        name="fused_block",
    )(A_x.reshape(S, D), A_wqkv, A_wo, B_w_gate.T, B_w_up.T, B_w_down)
    return out.reshape(1, S, D)
```

```python
import functools
import math

import jax
import jax.numpy as jnp
from jax import lax
import jax.experimental.pallas as pl
import jax.experimental.pallas.tpu as pltpu

S, D, H, DH, F = 2048, 640, 32, 20, 1728
T = 256
NB = S // T
NQT = T // 128
NG = H // 4
NP = H // 2
FT = F // 128
FM = FT * 128
NEG = -1e9
EPS = 1e-5
QSCALE = (DH ** -0.5) * math.log2(math.e)
f32, bf16 = jnp.float32, jnp.bfloat16

FA = 256
HEAD, TAIL1, TAIL2 = 3, 2, 2
HEAD0, TAIL10, TAIL20 = 0, 3, 4
KA, KB = 1, 3
WAIT_AT = 5
UNITS = ("q0", "k0", "q1", "k1", "q2", "v0", "v1", "v2", "k2")
LN_AT = (1, 9, 31)


def _ln(x):
    m = jnp.mean(x, axis=-1, keepdims=True)
    xc = x - m
    v = jnp.mean(xc * xc, axis=-1, keepdims=True)
    return xc * lax.rsqrt(v + EPS)


def _sel(mask, a, b):
    if a is None and b is None:
        return None
    if a is None:
        a = jnp.zeros_like(b)
    if b is None:
        b = jnp.zeros_like(a)
    return jnp.where(mask, a, b)


def _sigmoid(x):
    return 0.5 * jnp.tanh(0.5 * x) + 0.5


def _dot(a, b):
    return jnp.dot(a, b, precision=lax.Precision.DEFAULT, preferred_element_type=f32)


def _dot_nt(a, b):
    return lax.dot_general(a, b, (((1,), (1,)), ((), ())), precision=lax.Precision.DEFAULT,
                           preferred_element_type=f32)


def _proj_chunks(tiles, put, get):
    chunks = []

    def tail(group):
        def run():
            ns = {4: 1, 2: 2}.get(len(group), 4)
            for slot, (lhs, fn, _) in enumerate(group):
                a = lhs(512, D)
                q = a.shape[0] // ns
                put(slot, jnp.concatenate(
                    [fn(a[r * q:(r + 1) * q], 512, D) for r in range(ns)], axis=0))
        return run

    def head(slot, lhs, fn, done):
        def run():
            a = lhs(0, 512)
            done(get(slot, a.shape[0]) + fn(a, 0, 512))
        return run

    for i in range(0, len(tiles), 4):
        group = tiles[i:i + 4]
        chunks.append(tail(group))
        chunks += [head(slot, *tile) for slot, tile in enumerate(group)]
    return chunks


def _lazy_cols(fn):
    cache = []

    def get(k0, k1):
        if not cache:
            cache.append(fn())
        return cache[0][:, k0:k1]
    return get


def _kernel(x_hbm, wqkv_hbm, wo_hbm, wg_hbm, wu_hbm, wd_hbm, o_hbm,
            ob, xs, wqkv, wo, wgu, wd, sems,
            q_scr, k_scr, vt_scr, ot_scr, o_scr, h_scr, hn_scr, act_scr, *bufs):
    phase = pl.program_id(0)
    s_scr, g_scr = bufs[0:2], bufs[2]
    sets, xn_scr = [bufs[3:7], bufs[7:11]], bufs[11:14]
    a_scr = xn_scr
    zw = lax.shift_right_logical(phase, 8)
    zr = lax.shift_right_logical(phase, 9)

    def stage(k):
        def put(slot, val):
            sets[k][slot][zw, 0:val.shape[0]] = val

        def get(slot, n):
            return sets[k][slot][zr, 0:n]
        return put, get

    cp = pltpu.make_async_copy
    k1, k2 = D + 128 * KA, D + 128 * KB
    copies = dict(
        x0=cp(x_hbm.at[0:T], xs.at[0, 0:T], sems.at[0]),
        x1=cp(x_hbm.at[T:2 * T], xs.at[0, T:2 * T], sems.at[1]),
        wka=cp(wqkv_hbm.at[:, D:k1], wqkv.at[:, D:k1], sems.at[2]),
        wkb=cp(wqkv_hbm.at[:, k1:k2], wqkv.at[:, k1:k2], sems.at[3]),
        wkc=cp(wqkv_hbm.at[:, k2:2 * D], wqkv.at[:, k2:2 * D], sems.at[0]),
        wq=cp(wqkv_hbm.at[:, 0:D], wqkv.at[:, 0:D], sems.at[1]),
        wv=cp(wqkv_hbm.at[:, 2 * D:3 * D], wqkv.at[:, 2 * D:3 * D], sems.at[2]),
        wo=cp(wo_hbm, wo, sems.at[3]),
        wga=cp(wg_hbm.at[0:FA], wgu.at[0:FA], sems.at[3]),
        wua=cp(wu_hbm.at[0:FA], wgu.at[FM:FM + FA], sems.at[3]),
        x2=cp(x_hbm.at[2 * T:3 * T], xs.at[0, 2 * T:3 * T], sems.at[3]),
        x35=cp(x_hbm.at[3 * T:6 * T], xs.at[0, 3 * T:6 * T], sems.at[0]),
        wg2=cp(wg_hbm.at[FM:F], wgu.at[2 * FM:2 * FM + 64], sems.at[1]),
        wu2=cp(wu_hbm.at[FM:F], wgu.at[2 * FM + 64:2 * F], sems.at[1]),
        wgb=cp(wg_hbm.at[FA:FM], wgu.at[FA:FM], sems.at[1]),
        wub=cp(wu_hbm.at[FA:FM], wgu.at[FM + FA:2 * FM], sems.at[1]),
        wd=cp(wd_hbm, wd, sems.at[1]),
        x67=cp(x_hbm.at[6 * T:8 * T], xs.at[0, 6 * T:8 * T], sems.at[1]),
    )

    def rows_of(b, n=T):
        return pl.ds(b * T if isinstance(b, int) else pl.multiple_of(b * T, T), n)

    def ocopy(b):
        return cp(ob.at[rows_of(b)], o_hbm.at[rows_of(b)], sems.at[2])

    def ocopy_last(n):
        rows, cols = rows_of(NB - 1), pl.ds(n * 128, 128)
        return cp(ob.at[rows, cols], o_hbm.at[rows, cols], sems.at[2])

    lo4 = lax.broadcasted_iota(jnp.int32, (8, 128), 0) < 4

    def qkv_tiles(b, xn, which, hook=None, cs=tuple(range(NQT))):
        got = {}
        r0, nr = cs[0] * 128, len(cs) * 128
        lane = lax.broadcasted_iota(jnp.int32, (nr, 128), 1)

        def done(key, val):
            name, n = key
            if hook:
                hook(val)
            if name == "v":
                for c in cs:
                    vt = val[c * 128 - r0:(c + 1) * 128 - r0, :].T
                    for i in range(16):
                        p, e = divmod(16 * n + i, 5)
                        piece = vt[8 * i:8 * i + 8]
                        kt = b * NQT + c
                        if e == 2:
                            vt_scr[kt, 48 * p + 16:48 * p + 24, :] = jnp.where(lo4, piece, 1.0)
                            vt_scr[kt, 48 * p + 24:48 * p + 32, :] = jnp.where(lo4, 1.0, piece)
                        else:
                            o = 48 * p + 8 * (e if e < 2 else e + 1)
                            vt_scr[kt, o:o + 8, :] = piece
                return
            if name == "q":
                val = val * QSCALE
            got[key] = val
            for g in range(NG):
                lo = 80 * g
                t0, t1 = lo // 128, (lo + 79) // 128
                if t1 != n:
                    continue
                tile = val if t0 == t1 else jnp.where(lane >= lo % 128, got[(name, t0)], val)
                if name == "q":
                    q_scr.at[g, rows_of(b)][r0:r0 + nr, :] = tile
                else:
                    k_scr.at[g, rows_of(b)][r0:r0 + nr, :] = tile

        base = {"q": 0, "k": D, "v": 2 * D}
        tiles = []
        for name in which:
            for n in range(5):
                c0 = base[name] + 128 * n
                tiles.append((lambda k0, k1: xn(k0, k1)[r0:r0 + nr],
                              lambda a, k0, k1, c0=c0: _dot(a, wqkv[k0:k1, c0:c0 + 128]),
                              functools.partial(done, (name, n))))
        return tiles

    def ln1_part(b, r, part):
        rows = slice(part * T // 4, (part + 1) * T // 4)
        xn_scr[r][zw, rows, :] = _ln(xs.at[zr, rows_of(b)][rows, :].astype(f32))

    def gu_chunks(hn, head):
        def done(key, val):
            name, f = key
            if name == "g":
                g_scr[zw] = _sigmoid(val)
            elif name == "u":
                act_scr[:, f * 128:(f + 1) * 128] = g_scr[zr] * val
            else:
                act_scr[:, FM:F] = (_sigmoid(val) * pltpu.roll(val, 64, 1))[:, 0:64]

        tiles = []
        for f in range(FT):
            for name, r0 in (("g", f * 128), ("u", FM + f * 128)):
                tiles.append((hn, lambda a, k0, k1, r0=r0: _dot_nt(a, wgu[r0:r0 + 128, k0:k1]),
                              functools.partial(done, (name, f))))
        tiles.append((hn, lambda a, k0, k1: _dot_nt(a, wgu[2 * FM:2 * F, k0:k1]),
                      functools.partial(done, ("gu", FT))))
        return _proj_chunks(tiles[:FA // 64] if head else tiles[FA // 64:], *stage(0))

    def deferred(step, last=False):
        par = (step + 1) % 2

        def d_chunk(n0, n1, k0, k1, nsplit=1, then=None):
            def run():
                cols = slice(n0 * 128, n1 * 128)
                q = T // nsplit
                for r in range(nsplit):
                    rows = slice(r * q, (r + 1) * q)
                    y = h_scr[par, rows, cols] + _dot(act_scr[rows, k0:k1], wd[k0:k1, cols])
                    if k1 == F:
                        ob.at[rows_of(step - 1)][rows, cols] = y.astype(bf16)
                    else:
                        h_scr[par, rows, cols] = y
                if then:
                    then().start()
            return run

        early = [d_chunk(0, 2, 0, 256), d_chunk(2, 4, 0, 256), d_chunk(4, 5, 0, 256, 2)]
        ks = ((256, 768), (768, 1280), (1280, F))
        if last:
            late = [d_chunk(n, n + 1, k0, k1,
                            then=functools.partial(ocopy_last, n) if k1 == F else None)
                    for n in range(5) for k0, k1 in ks]
        else:
            late = [d_chunk(n, n + 1, k0, k1,
                            then=(lambda: ocopy(step - 1)) if (k1 == F and n == 4) else None)
                    for k0, k1 in ks for n in range(5)]
        return early + gu_chunks(_lazy_cols(lambda: hn_scr[...]), False) + late

    def main(step, dq):
        first = isinstance(step, int)
        blk = step
        lane32 = lax.broadcasted_iota(jnp.int32, (32, 128), 1)
        m_s1 = (lane32 & 32) != 0
        m_s2 = (lane32 & 64) != 0
        tri_first = lax.broadcasted_iota(jnp.int32, (32, 128), 0) > (lane32 & 31)
        kv = k_scr if first else k_scr.at[:, rows_of(step - 1, 2 * T)]
        koff = -T if first else 0
        qv = q_scr.at[:, rows_of(blk)]
        kt0 = blk * NQT
        tmin = lambda c: max(0, 8 - 4 * c) if first else 0
        soff = lambda c: -8 if first and c == 0 else 0

        def run(n, keep=0):
            for _ in range(n):
                if len(dq) > keep:
                    dq.pop(0)()

        def qk(c, g, buf):
            ms = {}
            for j in (3, 2, 1, 0):
                t0, t1 = max(j, tmin(c)), j + 9
                rows = (t1 - t0) * 32
                start = koff + c * 128 + t0 * 32
                qb = qv[g, c * 128 + j * 32:c * 128 + (j + 1) * 32, :]
                slots = []
                for s in range(4):
                    lo = (80 * g + 20 * (s ^ j)) % 128
                    slots.append(jnp.where(((lane32 - lo) & 127) < DH, qb, 0.0))
                qm = jnp.concatenate(slots, axis=0).astype(bf16)
                st = _dot_nt(kv[g, start:start + rows, :], qm)
                parts = []
                if t0 == j:
                    parts.append(jnp.where(tri_first, st[0:32], NEG))
                    parts.append(st[32:rows - 32])
                elif rows > 32:
                    parts.append(st[0:rows - 32])
                parts.append(jnp.where(tri_first, NEG, st[rows - 32:rows]))
                st = jnp.concatenate(parts, axis=0)
                ms[j] = jnp.max(st, axis=0, keepdims=True)
                s_scr[buf][zw, j, (t0 + soff(c)) * 32:(t1 + soff(c)) * 32, :] = st
            return ms

        def probs(c, kt, sbuf, ms):
            ph = [[] for _ in range(4)]
            for t in range(4 * kt, 4 * kt + 4):
                ts = t + soff(c)
                p = [jnp.exp2(s_scr[sbuf][zr, j, ts * 32:(ts + 1) * 32, :] - ms[j])
                     if j <= t <= j + 8 else None for j in range(4)]
                u = [_sel(m_s1, p[j ^ 1], p[j]) for j in range(4)]
                for h in range(4):
                    ph[h].append(_sel(m_s2, u[h ^ 2], u[h]))
            return [jnp.concatenate(ph[h], axis=0).astype(bf16) for h in range(4)]

        def pv(c, g, kt, sbuf, ms):
            ps = probs(c, kt, sbuf, ms)
            res = []
            for h in range(4):
                r0 = 48 * (2 * g + h // 2) + 24 * (h % 2)
                r = _dot(vt_scr[kt0 + c - 2 + kt, r0:r0 + 24, :], ps[h])
                if kt > tmin(c) // 4:
                    r = r + a_scr[kt - 1][zr, T:T + 24, h * 128:(h + 1) * 128]
                if kt < 2:
                    a_scr[kt][zw, T:T + 24, h * 128:(h + 1) * 128] = r
                res.append(r)
            if kt < 2:
                return
            for pp in range(2):
                re, ro = res[2 * pp], res[2 * pp + 1]
                a, b = re[16:24], ro[0:8]
                l = jnp.where(lo4, b, a)
                inv = pl.reciprocal(l, approx=True)
                inv = inv * (2.0 - l * inv)
                inv_r = pltpu.roll(inv, 4, 0)
                ie = jnp.where(lo4, inv_r, inv)
                io = jnp.where(lo4, inv, inv_r)
                mid = jnp.where(lo4, a, b) * inv_r
                pair = 2 * g + pp
                ot_scr[c, 40 * pair:40 * pair + 40, :] = jnp.concatenate(
                    [re[0:8] * ie, re[8:16] * ie, mid, ro[8:16] * io, ro[16:24] * io], axis=0)
            if g == NG - 1:
                finish(c)

        def finish(c):
            o = ot_scr[c].T
            hl = (lax.broadcasted_iota(jnp.int32, (32, D), 1) * 3277) >> 16
            h1 = (hl & 1) != 0
            h2 = (hl & 2) != 0
            b4 = [o[32 * j:32 * (j + 1)] for j in range(4)]
            u = [jnp.where(h1, b4[j ^ 1], b4[j]) for j in range(4)]
            out = [jnp.where(h2, u[j ^ 2], u[j]) for j in range(4)]
            o_scr[c * 128:(c + 1) * 128, :] = jnp.concatenate(out, axis=0).astype(bf16)

        if first:
            items = [((1, 0), g) for g in range(NG)]
        else:
            items = [((c,), g) for c in range(NQT) for g in range(NG)]
        n = len(items)
        head, tail1, tail2 = (HEAD0, TAIL10, TAIL20) if first else (HEAD, TAIL1, TAIL2)
        keep = tail1 + tail2
        run(head)
        navail = max(len(dq) - keep, 0)
        ms = {}
        for i in range(n + 1):
            if i < n:
                ms[i] = {c: qk(c, items[i][1], i % 2) for c in items[i][0]}
            nd = ((i + 1) * navail) // (n + 1) - (i * navail) // (n + 1)
            if i == 0:
                run(nd, keep)
                continue
            cs, g = items[i - 1]
            groups = [(c, kt) for c in cs for kt in range(tmin(c) // 4, 3)]
            pre = [0, 0, 0]
            for q in range(nd):
                pre[((2, 1, 0) if i < n else (0, 2, 1))[q % 3]] += 1
            for gi, ((c, kt), m) in enumerate(zip(groups, pre)):
                if first and gi == 2:
                    if i == WAIT_AT:
                        for name in ("wo", "wga", "wua", "x2"):
                            copies[name].wait()
                    if 0 <= i - WAIT_AT < 4:
                        ln1_part(2, 0, i - WAIT_AT)
                run(m, keep)
                pv(c, g, kt, (i - 1) % 2, ms[i - 1][c])
        run(tail1)

        hs = {}

        def h_done(n, val):
            hs[n] = xs[0, rows_of(blk), n * 128:(n + 1) * 128].astype(f32) + val
            h_scr[blk % 2, :, n * 128:(n + 1) * 128] = hs[n]

        o_cols = _lazy_cols(lambda: o_scr[...])
        tiles = [(o_cols, lambda a, k0, k1, n=n: _dot(a, wo[k0:k1, n * 128:(n + 1) * 128]),
                  functools.partial(h_done, n)) for n in range(5)]
        for ch in _proj_chunks(tiles, *stage(0)):
            ch()
        hn = _ln(jnp.concatenate([hs[n] for n in range(5)], axis=1)).astype(bf16)
        hn_scr[...] = hn
        run(len(dq))
        for ch in gu_chunks(lambda k0, k1: hn[:, k0:k1], True):
            ch()

    @pl.when(phase == 0)
    def _():
        def start(*names):
            for name in names:
                copies[name].start()

        start("x0", "x1", "wka", "wkb")

        def go(tiles):
            for ch in _proj_chunks(tiles, *stage(1)):
                ch()

        xn = []
        for b in range(2):
            copies["x%d" % b].wait()
            start(("wkc", "wq")[b])
            v = _ln(xs[0, rows_of(b), :].astype(f32)).astype(bf16)
            xn.append(lambda k0, k1, v=v: v[:, k0:k1])
        kt = [qkv_tiles(b, xn[b], "k") for b in range(2)]
        copies["wka"].wait()
        start("wv")
        go(kt[0][:KA] + kt[1][:KA])
        copies["wkb"].wait()
        start("wo", "wga", "wua", "x2")
        go(kt[0][KA:KB] + kt[1][KA:KB])
        copies["wkc"].wait()
        start("x35")
        go(kt[0][KB:] + kt[1][KB:])
        copies["wq"].wait()
        start("wg2", "wu2", "wgb", "wub", "wd", "x67")
        go(qkv_tiles(0, xn[0], "q"))
        copies["wv"].wait()
        go(qkv_tiles(0, xn[0], "v"))
        half = [t for name in "vq" for c in range(NQT) for t in qkv_tiles(1, xn[1], name, cs=(c,))]
        main(0, _proj_chunks(half, *stage(1)))
        copies["x35"].wait()

    def qkv3(step):
        lnq = {t0 + 2 * part: (r + 1, part) for r, t0 in enumerate(LN_AT) for part in range(4)}
        count = [0]

        def hook(val):
            job = lnq.pop(count[0], None)
            count[0] += 1
            if job:
                xs[zw, S:S + 16, 0:128] = val[0:16].astype(bf16)
                ln1_part(jnp.minimum(step + 1 + job[0], NB - 1), job[0] % 3, job[1])

        for name, r in UNITS:
            r = int(r)
            xn = lambda k0, k1, r=r: xn_scr[r][zr, 0:T, k0:k1]
            for ch in _proj_chunks(qkv_tiles(step + 1 + r, xn, name, hook), *stage(1)):
                ch()

    @pl.when(phase == 1)
    def _():
        def body(step, carry):
            @pl.when(jnp.logical_or(step == 1, step == 4))
            def _():
                qkv3(step)

                @pl.when(step == 1)
                def _():
                    for name in ("wg2", "wu2", "wgb", "wub", "wd", "x67"):
                        copies[name].wait()

            main(step, deferred(step))
            return carry

        lax.fori_loop(1, NB, body, 0)

    @pl.when(phase == 2)
    def _():
        for ch in deferred(NB, True):
            ch()
        cp(ob, o_hbm, sems.at[2]).wait()


@jax.jit
def pallas_sequential_preLN__sliding_block__glu_gated_glu__prompt_kernel(
    A_x: jax.Array,
    A_wqkv: jax.Array,
    A_wo: jax.Array,
    B_x: jax.Array,
    B_w_gate: jax.Array,
    B_w_up: jax.Array,
    B_w_down: jax.Array,
):
    del B_x
    hbm = pl.BlockSpec(memory_space=pl.ANY)
    out = pl.pallas_call(
        _kernel,
        grid=(3,),
        in_specs=[hbm] * 6,
        out_specs=hbm,
        out_shape=jax.ShapeDtypeStruct((S, D), bf16),
        scratch_shapes=[
            pltpu.VMEM((S, D), bf16),
            pltpu.VMEM((1, S + 64, D), bf16),
            pltpu.VMEM((D, 3 * D), bf16),
            pltpu.VMEM((D, D), bf16),
            pltpu.VMEM((2 * F, D), bf16),
            pltpu.VMEM((F, D), bf16),
            pltpu.SemaphoreType.DMA((4,)),
            pltpu.VMEM((NG, S, 128), f32),
            pltpu.VMEM((NG, S, 128), f32),
            pltpu.VMEM((S // 128, 48 * NP, 128), f32),
            pltpu.VMEM((NQT, D, 128), f32),
            pltpu.VMEM((T, D), bf16),
            pltpu.VMEM((2, T, D), f32),
            pltpu.VMEM((T, D), bf16),
            pltpu.VMEM((T, F), f32),
        ] + [pltpu.VMEM((1, 4, 384, 128), f32)] * 2
        + [pltpu.VMEM((1, T, 128), f32)] * 9
        + [pltpu.VMEM((1, T + 32, D), f32)] * 3,
        compiler_params=pltpu.CompilerParams(
            dimension_semantics=("arbitrary",),
            vmem_limit_bytes=100 * 1024 * 1024),
        name="fused_block",
    )(A_x.reshape(S, D), A_wqkv, A_wo, B_w_gate.T, B_w_up.T, B_w_down)
    return out.reshape(1, S, D)
```

```python
import functools
import math

import jax
import jax.numpy as jnp
from jax import lax
import jax.experimental.pallas as pl
import jax.experimental.pallas.tpu as pltpu

S, D, H, DH, F = 2048, 640, 32, 20, 1728
T = 256
NB = S // T
NQT = T // 128
NG = H // 4
NP = H // 2
FT = F // 128
FM = FT * 128
NEG = -1e9
EPS = 1e-5
QSCALE = (DH ** -0.5) * math.log2(math.e)
f32, bf16 = jnp.float32, jnp.bfloat16

FA = 256
HEAD, TAIL1, TAIL2 = 3, 2, 2
HEAD0, TAIL10, TAIL20 = 0, 3, 4
KA, KB = 1, 3
WAIT_AT = 5
UNITS = ("q0", "k0", "q1", "k1", "q2", "v0", "v1", "v2", "k2")
LN_AT = (1, 9, 31)


def _ln(x):
    m = jnp.mean(x, axis=-1, keepdims=True)
    xc = x - m
    v = jnp.mean(xc * xc, axis=-1, keepdims=True)
    return xc * lax.rsqrt(v + EPS)


def _sel(mask, a, b):
    if a is None and b is None:
        return None
    if a is None:
        a = jnp.zeros_like(b)
    if b is None:
        b = jnp.zeros_like(a)
    return jnp.where(mask, a, b)


def _sigmoid(x):
    return 0.5 * jnp.tanh(0.5 * x) + 0.5


def _dot(a, b):
    return jnp.dot(a, b, precision=lax.Precision.DEFAULT, preferred_element_type=f32)


def _dot_nt(a, b):
    return lax.dot_general(a, b, (((1,), (1,)), ((), ())), precision=lax.Precision.DEFAULT,
                           preferred_element_type=f32)


def _proj_chunks(tiles, put, get):
    chunks = []

    def tail(group):
        def run():
            ns = {4: 1, 2: 2}.get(len(group), 4)
            for slot, (lhs, fn, _) in enumerate(group):
                a = lhs(512, D)
                q = a.shape[0] // ns
                put(slot, jnp.concatenate(
                    [fn(a[r * q:(r + 1) * q], 512, D) for r in range(ns)], axis=0))
        return run

    def head(slot, lhs, fn, done):
        def run():
            a = lhs(0, 512)
            done(get(slot, a.shape[0]) + fn(a, 0, 512))
        return run

    for i in range(0, len(tiles), 4):
        group = tiles[i:i + 4]
        chunks.append(tail(group))
        chunks += [head(slot, *tile) for slot, tile in enumerate(group)]
    return chunks


def _lazy_cols(fn):
    cache = []

    def get(k0, k1):
        if not cache:
            cache.append(fn())
        return cache[0][:, k0:k1]
    return get


def _kernel(x_hbm, wqkv_hbm, wo_hbm, wg_hbm, wu_hbm, wd_hbm, o_hbm,
            ob, xs, wqkv, wo, wgu, wd, sems,
            q_scr, k_scr, vt_scr, ot_scr, o_scr, h_scr, hn_scr, act_scr, *bufs):
    pid = pl.program_id(0)
    s_scr, g_scr = bufs[0:2], bufs[2]
    sets, xn_scr = [bufs[3:7], bufs[7:11]], bufs[11:14]
    a_scr = xn_scr
    zw = lax.shift_right_logical(pid, 8)
    zr = lax.shift_right_logical(pid, 9)

    def stage(k):
        def put(slot, val):
            sets[k][slot][zw, 0:val.shape[0]] = val

        def get(slot, n):
            return sets[k][slot][zr, 0:n]
        return put, get

    cp = pltpu.make_async_copy
    k1, k2 = D + 128 * KA, D + 128 * KB
    copies = dict(
        x0=cp(x_hbm.at[0:T], xs.at[0, 0:T], sems.at[0]),
        x1=cp(x_hbm.at[T:2 * T], xs.at[0, T:2 * T], sems.at[1]),
        wka=cp(wqkv_hbm.at[:, D:k1], wqkv.at[:, D:k1], sems.at[2]),
        wkb=cp(wqkv_hbm.at[:, k1:k2], wqkv.at[:, k1:k2], sems.at[3]),
        wkc=cp(wqkv_hbm.at[:, k2:2 * D], wqkv.at[:, k2:2 * D], sems.at[0]),
        wq=cp(wqkv_hbm.at[:, 0:D], wqkv.at[:, 0:D], sems.at[1]),
        wv=cp(wqkv_hbm.at[:, 2 * D:3 * D], wqkv.at[:, 2 * D:3 * D], sems.at[2]),
        wo=cp(wo_hbm, wo, sems.at[3]),
        wga=cp(wg_hbm.at[0:FA], wgu.at[0:FA], sems.at[3]),
        wua=cp(wu_hbm.at[0:FA], wgu.at[FM:FM + FA], sems.at[3]),
        x2=cp(x_hbm.at[2 * T:3 * T], xs.at[0, 2 * T:3 * T], sems.at[3]),
        x35=cp(x_hbm.at[3 * T:6 * T], xs.at[0, 3 * T:6 * T], sems.at[0]),
        wg2=cp(wg_hbm.at[FM:F], wgu.at[2 * FM:2 * FM + 64], sems.at[1]),
        wu2=cp(wu_hbm.at[FM:F], wgu.at[2 * FM + 64:2 * F], sems.at[1]),
        wgb=cp(wg_hbm.at[FA:FM], wgu.at[FA:FM], sems.at[1]),
        wub=cp(wu_hbm.at[FA:FM], wgu.at[FM + FA:2 * FM], sems.at[1]),
        wd=cp(wd_hbm, wd, sems.at[1]),
        x67=cp(x_hbm.at[6 * T:8 * T], xs.at[0, 6 * T:8 * T], sems.at[1]),
    )

    def rows_of(b, n=T):
        return pl.ds(b * T if isinstance(b, int) else pl.multiple_of(b * T, T), n)

    def ocopy(b):
        return cp(ob.at[rows_of(b)], o_hbm.at[rows_of(b)], sems.at[2])

    def ocopy_last(n):
        rows, cols = rows_of(NB - 1), pl.ds(n * 128, 128)
        return cp(ob.at[rows, cols], o_hbm.at[rows, cols], sems.at[2])

    lo4 = lax.broadcasted_iota(jnp.int32, (8, 128), 0) < 4

    def qkv_tiles(b, xn, which, hook=None, cs=tuple(range(NQT))):
        got = {}
        r0, nr = cs[0] * 128, len(cs) * 128
        lane = lax.broadcasted_iota(jnp.int32, (nr, 128), 1)

        def done(key, val):
            name, n = key
            if hook:
                hook(val)
            if name == "v":
                for c in cs:
                    vt = val[c * 128 - r0:(c + 1) * 128 - r0, :].T
                    for i in range(16):
                        p, e = divmod(16 * n + i, 5)
                        piece = vt[8 * i:8 * i + 8]
                        kt = b * NQT + c
                        if e == 2:
                            vt_scr[kt, 48 * p + 16:48 * p + 24, :] = jnp.where(lo4, piece, 1.0)
                            vt_scr[kt, 48 * p + 24:48 * p + 32, :] = jnp.where(lo4, 1.0, piece)
                        else:
                            o = 48 * p + 8 * (e if e < 2 else e + 1)
                            vt_scr[kt, o:o + 8, :] = piece
                return
            if name == "q":
                val = val * QSCALE
            got[key] = val
            for g in range(NG):
                lo = 80 * g
                t0, t1 = lo // 128, (lo + 79) // 128
                if t1 != n:
                    continue
                tile = val if t0 == t1 else jnp.where(lane >= lo % 128, got[(name, t0)], val)
                if name == "q":
                    q_scr.at[g, rows_of(b)][r0:r0 + nr, :] = tile
                else:
                    k_scr.at[g, rows_of(b)][r0:r0 + nr, :] = tile

        base = {"q": 0, "k": D, "v": 2 * D}
        tiles = []
        for name in which:
            for n in range(5):
                c0 = base[name] + 128 * n
                tiles.append((lambda k0, k1: xn(k0, k1)[r0:r0 + nr],
                              lambda a, k0, k1, c0=c0: _dot(a, wqkv[k0:k1, c0:c0 + 128]),
                              functools.partial(done, (name, n))))
        return tiles

    def ln1_part(b, r, part):
        rows = slice(part * T // 4, (part + 1) * T // 4)
        xn_scr[r][zw, rows, :] = _ln(xs.at[zr, rows_of(b)][rows, :].astype(f32))

    def gu_chunks(hn, head):
        def done(key, val):
            name, f = key
            if name == "g":
                g_scr[zw] = _sigmoid(val)
            elif name == "u":
                act_scr[:, f * 128:(f + 1) * 128] = g_scr[zr] * val
            else:
                act_scr[:, FM:F] = (_sigmoid(val) * pltpu.roll(val, 64, 1))[:, 0:64]

        tiles = []
        for f in range(FT):
            for name, r0 in (("g", f * 128), ("u", FM + f * 128)):
                tiles.append((hn, lambda a, k0, k1, r0=r0: _dot_nt(a, wgu[r0:r0 + 128, k0:k1]),
                              functools.partial(done, (name, f))))
        tiles.append((hn, lambda a, k0, k1: _dot_nt(a, wgu[2 * FM:2 * F, k0:k1]),
                      functools.partial(done, ("gu", FT))))
        return _proj_chunks(tiles[:FA // 64] if head else tiles[FA // 64:], *stage(0))

    def deferred(step, last=False):
        par = (step + 1) % 2

        def d_chunk(n0, n1, k0, k1, nsplit=1, then=None):
            def run():
                cols = slice(n0 * 128, n1 * 128)
                q = T // nsplit
                for r in range(nsplit):
                    rows = slice(r * q, (r + 1) * q)
                    y = h_scr[par, rows, cols] + _dot(act_scr[rows, k0:k1], wd[k0:k1, cols])
                    if k1 == F:
                        ob.at[rows_of(step - 1)][rows, cols] = y.astype(bf16)
                    else:
                        h_scr[par, rows, cols] = y
                if then:
                    then().start()
            return run

        early = [d_chunk(0, 2, 0, 256), d_chunk(2, 4, 0, 256), d_chunk(4, 5, 0, 256, 2)]
        ks = ((256, 768), (768, 1280), (1280, F))
        if last:
            late = [d_chunk(n, n + 1, k0, k1,
                            then=functools.partial(ocopy_last, n) if k1 == F else None)
                    for n in range(5) for k0, k1 in ks]
        else:
            late = [d_chunk(n, n + 1, k0, k1,
                            then=(lambda: ocopy(step - 1)) if (k1 == F and n == 4) else None)
                    for k0, k1 in ks for n in range(5)]
        return early + gu_chunks(_lazy_cols(lambda: hn_scr[...]), False) + late

    def main(step, dq):
        first = isinstance(step, int)
        blk = step
        lane32 = lax.broadcasted_iota(jnp.int32, (32, 128), 1)
        m_s1 = (lane32 & 32) != 0
        m_s2 = (lane32 & 64) != 0
        tri_first = lax.broadcasted_iota(jnp.int32, (32, 128), 0) > (lane32 & 31)
        kv = k_scr if first else k_scr.at[:, rows_of(step - 1, 2 * T)]
        koff = -T if first else 0
        qv = q_scr.at[:, rows_of(blk)]
        kt0 = blk * NQT
        tmin = lambda c: max(0, 8 - 4 * c) if first else 0
        soff = lambda c: -8 if first and c == 0 else 0

        def run(n, keep=0):
            for _ in range(n):
                if len(dq) > keep:
                    dq.pop(0)()

        def qk(c, g, buf):
            ms = {}
            for j in (3, 2, 1, 0):
                t0, t1 = max(j, tmin(c)), j + 9
                rows = (t1 - t0) * 32
                start = koff + c * 128 + t0 * 32
                qb = qv[g, c * 128 + j * 32:c * 128 + (j + 1) * 32, :]
                slots = []
                for s in range(4):
                    lo = (80 * g + 20 * (s ^ j)) % 128
                    slots.append(jnp.where(((lane32 - lo) & 127) < DH, qb, 0.0))
                qm = jnp.concatenate(slots, axis=0).astype(bf16)
                st = _dot_nt(kv[g, start:start + rows, :], qm)
                parts = []
                if t0 == j:
                    parts.append(jnp.where(tri_first, st[0:32], NEG))
                    parts.append(st[32:rows - 32])
                elif rows > 32:
                    parts.append(st[0:rows - 32])
                parts.append(jnp.where(tri_first, NEG, st[rows - 32:rows]))
                st = jnp.concatenate(parts, axis=0)
                ms[j] = jnp.max(st, axis=0, keepdims=True)
                s_scr[buf][zw, j, (t0 + soff(c)) * 32:(t1 + soff(c)) * 32, :] = st
            return ms

        def probs(c, kt, sbuf, ms):
            ph = [[] for _ in range(4)]
            for t in range(4 * kt, 4 * kt + 4):
                ts = t + soff(c)
                p = [jnp.exp2(s_scr[sbuf][zr, j, ts * 32:(ts + 1) * 32, :] - ms[j])
                     if j <= t <= j + 8 else None for j in range(4)]
                u = [_sel(m_s1, p[j ^ 1], p[j]) for j in range(4)]
                for h in range(4):
                    ph[h].append(_sel(m_s2, u[h ^ 2], u[h]))
            return [jnp.concatenate(ph[h], axis=0).astype(bf16) for h in range(4)]

        def pv(c, g, kt, sbuf, ms):
            ps = probs(c, kt, sbuf, ms)
            res = []
            for h in range(4):
                r0 = 48 * (2 * g + h // 2) + 24 * (h % 2)
                r = _dot(vt_scr[kt0 + c - 2 + kt, r0:r0 + 24, :], ps[h])
                if kt > tmin(c) // 4:
                    r = r + a_scr[kt - 1][zr, T:T + 24, h * 128:(h + 1) * 128]
                if kt < 2:
                    a_scr[kt][zw, T:T + 24, h * 128:(h + 1) * 128] = r
                res.append(r)
            if kt < 2:
                return
            for pp in range(2):
                re, ro = res[2 * pp], res[2 * pp + 1]
                a, b = re[16:24], ro[0:8]
                l = jnp.where(lo4, b, a)
                inv = pl.reciprocal(l, approx=True)
                inv = inv * (2.0 - l * inv)
                inv_r = pltpu.roll(inv, 4, 0)
                ie = jnp.where(lo4, inv_r, inv)
                io = jnp.where(lo4, inv, inv_r)
                mid = jnp.where(lo4, a, b) * inv_r
                pair = 2 * g + pp
                ot_scr[c, 40 * pair:40 * pair + 40, :] = jnp.concatenate(
                    [re[0:8] * ie, re[8:16] * ie, mid, ro[8:16] * io, ro[16:24] * io], axis=0)
            if g == NG - 1:
                finish(c)

        def finish(c):
            o = ot_scr[c].T
            hl = (lax.broadcasted_iota(jnp.int32, (32, D), 1) * 3277) >> 16
            h1 = (hl & 1) != 0
            h2 = (hl & 2) != 0
            b4 = [o[32 * j:32 * (j + 1)] for j in range(4)]
            u = [jnp.where(h1, b4[j ^ 1], b4[j]) for j in range(4)]
            out = [jnp.where(h2, u[j ^ 2], u[j]) for j in range(4)]
            o_scr[c * 128:(c + 1) * 128, :] = jnp.concatenate(out, axis=0).astype(bf16)

        if first:
            items = [((1, 0), g) for g in range(NG)]
        else:
            items = [((c,), g) for c in range(NQT) for g in range(NG)]
        n = len(items)
        head, tail1, tail2 = (HEAD0, TAIL10, TAIL20) if first else (HEAD, TAIL1, TAIL2)
        keep = tail1 + tail2
        run(head)
        navail = max(len(dq) - keep, 0)
        ms = {}
        for i in range(n + 1):
            if i < n:
                ms[i] = {c: qk(c, items[i][1], i % 2) for c in items[i][0]}
            nd = ((i + 1) * navail) // (n + 1) - (i * navail) // (n + 1)
            if i == 0:
                run(nd, keep)
                continue
            cs, g = items[i - 1]
            groups = [(c, kt) for c in cs for kt in range(tmin(c) // 4, 3)]
            pre = [0, 0, 0]
            for q in range(nd):
                pre[((2, 1, 0) if i < n else (0, 2, 1))[q % 3]] += 1
            for gi, ((c, kt), m) in enumerate(zip(groups, pre)):
                if first and gi == 2:
                    if i == WAIT_AT:
                        for name in ("wo", "wga", "wua", "x2"):
                            copies[name].wait()
                    if 0 <= i - WAIT_AT < 4:
                        ln1_part(2, 0, i - WAIT_AT)
                run(m, keep)
                pv(c, g, kt, (i - 1) % 2, ms[i - 1][c])
        run(tail1)

        hs = {}

        def h_done(n, val):
            hs[n] = xs[0, rows_of(blk), n * 128:(n + 1) * 128].astype(f32) + val
            h_scr[blk % 2, :, n * 128:(n + 1) * 128] = hs[n]

        o_cols = _lazy_cols(lambda: o_scr[...])
        tiles = [(o_cols, lambda a, k0, k1, n=n: _dot(a, wo[k0:k1, n * 128:(n + 1) * 128]),
                  functools.partial(h_done, n)) for n in range(5)]
        for ch in _proj_chunks(tiles, *stage(0)):
            ch()
        hn = _ln(jnp.concatenate([hs[n] for n in range(5)], axis=1)).astype(bf16)
        hn_scr[...] = hn
        run(len(dq))
        for ch in gu_chunks(lambda k0, k1: hn[:, k0:k1], True):
            ch()

    @pl.when(pid == 0)
    def _():
        def start(*names):
            for name in names:
                copies[name].start()

        start("x0", "x1", "wka", "wkb")

        def go(tiles):
            for ch in _proj_chunks(tiles, *stage(1)):
                ch()

        xn = []
        for b in range(2):
            copies["x%d" % b].wait()
            start(("wkc", "wq")[b])
            v = _ln(xs[0, rows_of(b), :].astype(f32)).astype(bf16)
            xn.append(lambda k0, k1, v=v: v[:, k0:k1])
        kt = [qkv_tiles(b, xn[b], "k") for b in range(2)]
        copies["wka"].wait()
        start("wv")
        go(kt[0][:KA] + kt[1][:KA])
        copies["wkb"].wait()
        start("wo", "wga", "wua", "x2")
        go(kt[0][KA:KB] + kt[1][KA:KB])
        copies["wkc"].wait()
        start("x35")
        go(kt[0][KB:] + kt[1][KB:])
        copies["wq"].wait()
        start("wg2", "wu2", "wgb", "wub", "wd", "x67")
        go(qkv_tiles(0, xn[0], "q"))
        copies["wv"].wait()
        go(qkv_tiles(0, xn[0], "v"))
        half = [t for name in "vq" for c in range(NQT) for t in qkv_tiles(1, xn[1], name, cs=(c,))]
        main(0, _proj_chunks(half, *stage(1)))
        copies["x35"].wait()

    def qkv3(step):
        lnq = {t0 + 2 * part: (r + 1, part) for r, t0 in enumerate(LN_AT) for part in range(4)}
        count = [0]

        def hook(val):
            job = lnq.pop(count[0], None)
            count[0] += 1
            if job:
                xs[zw, S:S + 16, 0:128] = val[0:16].astype(bf16)
                ln1_part(jnp.minimum(step + 1 + job[0], NB - 1), job[0] % 3, job[1])

        for name, r in UNITS:
            r = int(r)
            xn = lambda k0, k1, r=r: xn_scr[r][zr, 0:T, k0:k1]
            for ch in _proj_chunks(qkv_tiles(step + 1 + r, xn, name, hook), *stage(1)):
                ch()

    @pl.when(jnp.logical_or(pid == 1, pid == 4))
    def _():
        qkv3(pid)

        @pl.when(pid == 1)
        def _():
            for name in ("wg2", "wu2", "wgb", "wub", "wd", "x67"):
                copies[name].wait()

    @pl.when(jnp.logical_and(pid > 0, pid < NB))
    def _():
        main(pid, deferred(pid))

    @pl.when(pid == NB)
    def _():
        for ch in deferred(NB, True):
            ch()
        cp(ob, o_hbm, sems.at[2]).wait()


@jax.jit
def pallas_sequential_preLN__sliding_block__glu_gated_glu__prompt_kernel(
    A_x: jax.Array,
    A_wqkv: jax.Array,
    A_wo: jax.Array,
    B_x: jax.Array,
    B_w_gate: jax.Array,
    B_w_up: jax.Array,
    B_w_down: jax.Array,
):
    del B_x
    hbm = pl.BlockSpec(memory_space=pl.ANY)
    out = pl.pallas_call(
        _kernel,
        grid=(NB + 1,),
        in_specs=[hbm] * 6,
        out_specs=hbm,
        out_shape=jax.ShapeDtypeStruct((S, D), bf16),
        scratch_shapes=[
            pltpu.VMEM((S, D), bf16),
            pltpu.VMEM((1, S + 64, D), bf16),
            pltpu.VMEM((D, 3 * D), bf16),
            pltpu.VMEM((D, D), bf16),
            pltpu.VMEM((2 * F, D), bf16),
            pltpu.VMEM((F, D), bf16),
            pltpu.SemaphoreType.DMA((4,)),
            pltpu.VMEM((NG, S, 128), f32),
            pltpu.VMEM((NG, S, 128), f32),
            pltpu.VMEM((S // 128, 48 * NP, 128), f32),
            pltpu.VMEM((NQT, D, 128), f32),
            pltpu.VMEM((T, D), bf16),
            pltpu.VMEM((2, T, D), f32),
            pltpu.VMEM((T, D), bf16),
            pltpu.VMEM((T, F), f32),
        ] + [pltpu.VMEM((1, 4, 384, 128), f32)] * 2
        + [pltpu.VMEM((1, T, 128), f32)] * 9
        + [pltpu.VMEM((1, T + 32, D), f32)] * 3,
        compiler_params=pltpu.CompilerParams(
            dimension_semantics=("arbitrary",),
            vmem_limit_bytes=100 * 1024 * 1024),
        name="fused_block",
    )(A_x.reshape(S, D), A_wqkv, A_wo, B_w_gate.T, B_w_up.T, B_w_down)
    return out.reshape(1, S, D)
```
